```python
import jax
import jax.numpy as jnp

def _softmax(x, axis=-1):
    return jax.nn.softmax(x, axis=axis)

def _gelu(x):
    return jax.nn.gelu(x, approximate=True)

def _silu(x):
    return jax.nn.silu(x)

def _sigmoid(x):
    return jax.nn.sigmoid(x)

def _layernorm(x, axis=-1, eps=1e-05):
    m = jnp.mean(x, axis=axis, keepdims=True)
    v = jnp.var(x, axis=axis, keepdims=True)
    return (x - m) / jnp.sqrt(v + eps)

def _scatter_add(tgt, idx, src, axis=0):
    return tgt.at[idx].add(src)

def _segment_sum(src, seg, n):
    return jax.ops.segment_sum(src, seg, n)

class _Rng:

    def __init__(self, key):
        self._k = key

    def _next(self):
        self._k, sub = jax.random.split(self._k)
        return sub

    def normal(self, shape):
        return jax.random.normal(self._next(), shape, dtype=jnp.bfloat16)

    def randint(self, lo, hi, shape):
        return jax.random.randint(self._next(), shape, lo, hi, dtype=jnp.int32)

    def uniform(self, shape, lo=0.0, hi=1.0):
        return jax.random.uniform(self._next(), shape, jnp.bfloat16, lo, hi)

    def permutation(self, n):
        return jax.random.permutation(self._next(), n)
kernel_name = 'gated_mix__memory_aug_recurrent_mem_tr__sliding_local_dilated__prompt'

def setup_inputs():
    _rng = _Rng(jax.random.key(int.from_bytes(__import__("os").urandom(4), "little")))
    _w = lambda a: (lambda t: t.astype(jnp.bfloat16) if jnp.issubdtype(t.dtype, jnp.floating) else t)(jnp.asarray(a))

    def _A_setup():
        B, S, Dm = (1, 2048, 640)
        H, Dh = (32, 192)
        M, seg = (8, 32)
        seg = min(seg, S)
        S = S // seg * seg
        return {'x': _w((lambda *s: _rng.normal(s) * 0.05)(B, S, Dm)), 'mem0': _w((lambda *s: _rng.normal(s) * 0.05)(B, M, Dm)), 'Wq': _w((lambda *s: _rng.normal(s) * 0.05)(Dm, H, Dh) * Dm ** (-0.5)), 'Wk': _w((lambda *s: _rng.normal(s) * 0.05)(Dm, H, Dh) * Dm ** (-0.5)), 'Wv': _w((lambda *s: _rng.normal(s) * 0.05)(Dm, H, Dh) * Dm ** (-0.5)), 'Wo': _w((lambda *s: _rng.normal(s) * 0.05)(H, Dh, Dm) * (H * Dh) ** (-0.5)), 'seg_len': seg}
    _A_in = _A_setup()

    def _B_setup():
        B, S, D = (1, 2048, 640)
        return {'x': _w((lambda *s: _rng.normal(s) * 0.05)(B, S, D)), 'wqkv': _w((lambda *s: _rng.normal(s) * 0.05)(D, 3 * D)), 'wo': _w((lambda *s: _rng.normal(s) * 0.05)(D, D))}
    _B_in = _B_setup()
    return {'A_x': _A_in['x'], 'A_mem0': _A_in['mem0'], 'A_Wq': _A_in['Wq'], 'A_Wk': _A_in['Wk'], 'A_Wv': _A_in['Wv'], 'A_Wo': _A_in['Wo'], 'A_seg_len': _A_in['seg_len'], 'B_x': _B_in['x'], 'B_wqkv': _B_in['wqkv'], 'B_wo': _B_in['wo'], 'gate_w': _w((lambda *s: _rng.normal(s) * 0.05)(640))}

def reference(A_x, A_mem0, A_Wq, A_Wk, A_Wv, A_Wo, A_seg_len, B_x, B_wqkv, B_wo, gate_w):

    def _A_ref(x, mem0, Wq, Wk, Wv, Wo, seg_len):
        B, S, Dm = x.shape
        H, Dh = (Wq.shape[1], Wq.shape[2])
        M = mem0.shape[1]
        scale = Dh ** (-0.5)
        n_seg = S // seg_len
        L = M + seg_len
        idx = jnp.arange(L)
        mask = (idx[:, None] < M) | (idx[:, None] >= idx[None, :])
        mem = mem0
        outs = []
        for s in range(n_seg):
            xs = x[:, s * seg_len:(s + 1) * seg_len, :].copy()
            h = jnp.concatenate([mem, xs], axis=1)
            q = jnp.einsum('btd,dhe->bhte', h, Wq)
            k = jnp.einsum('btd,dhe->bhte', h, Wk)
            v = jnp.einsum('btd,dhe->bhte', h, Wv)
            scores = jnp.einsum('bhqe,bhke->bhqk', q, k) * scale
            scores = jnp.where(mask[None, None], scores, -1000000000.0)
            p = _softmax(scores, axis=-1)
            o = jnp.einsum('bhqk,bhke->bhqe', p, v)
            o = jnp.einsum('bhte,hed->btd', o, Wo)
            mem = o[:, :M, :].copy()
            outs.append(o[:, M:, :])
        return jnp.concatenate(outs, axis=1)

    def _B_ref(x, wqkv, wo):
        B, S, D = x.shape
        H = 32
        Dh = D // H
        W, dil = (8, 2)
        qkv = (lambda x, *d: x.transpose(*d))((x @ wqkv).reshape(B, S, 3, H, Dh), 2, 0, 3, 1, 4)
        q, k, v = (qkv[0], qkv[1], qkv[2])
        scale = Dh ** (-0.5)
        pos = jnp.arange(S)
        off = jnp.arange(W) * dil
        idx = pos[:, None] - off[None, :]
        mask = idx >= 0
        idx_c = jnp.where(mask, idx, 0).reshape(-1)
        kg = k[:, :, idx_c, :].reshape(B, H, S, W, Dh)
        vg = v[:, :, idx_c, :].reshape(B, H, S, W, Dh)
        logits = jnp.einsum('bhsd,bhswd->bhsw', q, kg) * scale
        logits = jnp.where(mask[None, None, :, :], logits, -1000000000.0)
        attn = _softmax(logits, axis=-1)
        o = jnp.einsum('bhsw,bhswd->bhsd', attn, vg)
        return (lambda x, *d: x.transpose(*d))(o, 0, 2, 1, 3).reshape(B, S, D) @ wo
    x = A_x
    g = _sigmoid((x * gate_w).sum(-1, keepdims=True))
    a = _A_ref(x, A_mem0, A_Wq, A_Wk, A_Wv, A_Wo, A_seg_len)
    b = _B_ref(x, B_wqkv, B_wo)
    return g * a + (1 - g) * b
```

```python
import functools

import jax
import jax.numpy as jnp
import jax.experimental.pallas as pl
import jax.experimental.pallas.tpu as pltpu

F32 = jnp.float32
BF16 = jnp.bfloat16
U32 = jnp.uint32
NEG = -1000000000.0

B_HEADS = 32
B_WIN = 8
B_DIL = 2
HALO = 16
RB = 256
RS = 16
LANES = 128
LAG1, LAG2, LAG3 = 2, 4, 8


def _iota(shape, dim):
    return jax.lax.broadcasted_iota(jnp.int32, shape, dim)


def _dot(a, b):
    return jnp.dot(a, b, preferred_element_type=F32)


def _dot_nt(a, b):
    return jax.lax.dot_general(a, b, (((1,), (1,)), ((), ())), preferred_element_type=F32)


def _kernel(x_hbm, mem0_ref, wq_hbm, wk_hbm, wv_hbm, wo_hbm, bqkv_hbm, bwo_hbm, gw_ref,
            out_hbm,
            x_vm, bqkv_vm, bwo_vm, bqkv_p, bwo_p, stage, wqkv_s, wo_s,
            q_b, k_b, v_b, o_b, bmix, gate, out_vm, in_sem, w_sem, out_sem,
            *, seg, dh):
    S, D = x_vm.shape
    M = mem0_ref.shape[0]
    L = M + seg
    n_seg = S // seg
    PW = 2 * dh
    n_pair = wo_hbm.shape[0] // PW
    n_blk = S // RB
    ppb = n_pair // n_blk
    nt = D // LANES
    bdh = D // B_HEADS

    cp_bqkv = pltpu.make_async_copy(bqkv_hbm, bqkv_vm, in_sem.at[0])
    cp_x = pltpu.make_async_copy(x_hbm, x_vm, in_sem.at[1])
    cp_bwo = pltpu.make_async_copy(bwo_hbm, bwo_vm, in_sem.at[2])
    cp_bqkv.start()
    cp_x.start()
    cp_bwo.start()

    def w_copies(g):
        rows = pl.ds(pl.multiple_of(g * PW, PW), PW)
        return [pltpu.make_async_copy(src.at[rows, :], stage.at[g, j], w_sem.at[g, j])
                for j, src in enumerate((wq_hbm, wk_hbm, wv_hbm, wo_hbm))]

    def start_block_weights(i):
        for t in range(ppb):
            for c in w_copies(i * ppb + t):
                c.start()

    r = _iota((D, D), 0)
    c = _iota((D, D), 1)
    perm = jnp.where(r == (c % B_HEADS) * bdh + c // B_HEADS, 1.0, 0.0).astype(BF16)
    cp_bqkv.wait()
    start_block_weights(0)
    for j in range(3):
        bqkv_p[:, j * D:(j + 1) * D] = _dot(bqkv_vm[:, j * D:(j + 1) * D], perm).astype(BF16)
    cp_bwo.wait()
    wide = bwo_vm[...].astype(F32)
    for t in range(nt):
        k_b[t, 0:D, :] = wide[:, t * LANES:(t + 1) * LANES]
    for d in range(bdh):
        for t in range(nt):
            bwo_p[d * B_HEADS:(d + 1) * B_HEADS, t * LANES:(t + 1) * LANES] = (
                k_b[t, pl.ds(d, B_HEADS, stride=bdh), :].astype(BF16))
    cp_x.wait()

    gw = gw_ref[...].astype(F32)
    b_scale = bdh ** -0.5

    def relayout(g):
        for c in w_copies(g):
            c.wait()
        for j in range(3):
            wt = stage[g, j].T
            wqkv_s[g, :, j * PW:(j + 1) * PW] = pltpu.bitcast(wt, U32)
        wo_s[g] = pltpu.bitcast(stage[g, 3], U32)

    def b_block(i, carry):
        @pl.when(i + 1 < n_blk)
        def _():
            start_block_weights(i + 1)

        row0 = pl.multiple_of(i * RB, RB)
        xb = x_vm[pl.ds(row0, RB), :]
        q = _dot(xb, bqkv_p[:, 0:D]) * b_scale
        k = _dot(xb, bqkv_p[:, D:2 * D])
        v = _dot(xb, bqkv_p[:, 2 * D:3 * D])
        q_b[...] = q
        for t in range(nt):
            k_b[t, HALO:HALO + RB, :] = k[:, t * LANES:(t + 1) * LANES]
            v_b[t, HALO:HALO + RB, :] = v[:, t * LANES:(t + 1) * LANES]

        @pl.when(i == 0)
        def _():
            for t in range(nt):
                k_b[t, 0:HALO, :] = jnp.broadcast_to(k_b[t, HALO:HALO + 1, :], (HALO, LANES))
                v_b[t, 0:HALO, :] = jnp.broadcast_to(v_b[t, HALO:HALO + 1, :], (HALO, LANES))

        for sb in range(RB // RS):
            base = HALO + sb * RS
            qs = [q_b[sb * RS:(sb + 1) * RS, t * LANES:(t + 1) * LANES] for t in range(nt)]
            logits = []
            for w in range(B_WIN):
                lo = base - w * B_DIL
                acc = qs[0] * k_b[0, lo:lo + RS, :]
                for t in range(1, nt):
                    acc = acc + qs[t] * k_b[t, lo:lo + RS, :]
                acc = acc + pltpu.roll(acc, 64, 1)
                acc = acc + pltpu.roll(acc, 32, 1)
                if sb * RS < w * B_DIL:
                    pos = row0 + sb * RS + _iota((RS, LANES), 0)
                    acc = jnp.where(pos >= w * B_DIL, acc, NEG)
                logits.append(acc)
            mx = functools.reduce(jnp.maximum, logits)
            es = [jnp.exp(l - mx) for l in logits]
            inv = 1.0 / functools.reduce(jnp.add, es)
            ps = [e * inv for e in es]
            for t in range(nt):
                acc = ps[0] * v_b[t, base:base + RS, :]
                for w in range(1, B_WIN):
                    lo = base - w * B_DIL
                    acc = acc + ps[w] * v_b[t, lo:lo + RS, :]
                o_b[sb * RS:(sb + 1) * RS, t * LANES:(t + 1) * LANES] = acc.astype(BF16)

        for t in range(nt):
            k_b[t, 0:HALO, :] = k_b[t, RB:RB + HALO, :]
            v_b[t, 0:HALO, :] = v_b[t, RB:RB + HALO, :]

        b = _dot(o_b[...], bwo_p[...])
        z = jnp.sum(xb.astype(F32) * gw, axis=1, keepdims=True)
        g = 1.0 / (1.0 + jnp.exp(-z))
        gate[pl.ds(row0, RB), :] = jnp.broadcast_to(g, (RB, LANES))
        bmix[pl.ds(row0, RB), :] = (1.0 - g) * b

        for t in range(ppb):
            relayout(i * ppb + t)
        return carry

    jax.lax.fori_loop(0, n_blk, b_block, 0)

    a_scale = dh ** -0.5
    half = dh - LANES

    def out_copy(s):
        rows = pl.ds(pl.multiple_of(s * seg, seg), seg)
        return pltpu.make_async_copy(out_vm.at[rows, :], out_hbm.at[rows, :], out_sem.at[0])

    def block_diag(a):
        lo = _iota((L, LANES), 1) < half
        z = jnp.zeros((L, LANES), F32)
        mid = a[:, LANES:2 * LANES]
        top = jnp.concatenate([a[:, 0:LANES], jnp.where(lo, mid, 0.0), z], axis=1)
        bot = jnp.concatenate([z, jnp.where(lo, 0.0, mid), a[:, 2 * LANES:3 * LANES]], axis=1)
        return jnp.concatenate([top, bot], axis=0).astype(BF16)

    def a_step(s, mem):
        row0 = pl.multiple_of(s * seg, seg)
        h = jnp.concatenate([mem, x_vm[pl.ds(row0, seg), :].astype(F32)], axis=0)
        row = _iota((L, 2 * L), 0)
        col = _iota((L, 2 * L), 1)
        first = col < L
        key = jnp.where(first, col, col - L)
        visible = (row < M) | (row >= key)

        def project(g):
            return _dot(h, pltpu.bitcast(wqkv_s[g], BF16))

        def probs(qkv):
            sc = _dot_nt(qkv[:, 0:PW], block_diag(qkv[:, PW:2 * PW])) * a_scale
            sc = jnp.where(visible, sc, NEG)
            m0 = jnp.max(jnp.where(first, sc, -jnp.inf), axis=1, keepdims=True)
            m1 = jnp.max(jnp.where(first, -jnp.inf, sc), axis=1, keepdims=True)
            e = jnp.exp(sc - jnp.where(first, m0, m1))
            s0 = jnp.sum(jnp.where(first, e, 0.0), axis=1, keepdims=True)
            s1 = jnp.sum(jnp.where(first, 0.0, e), axis=1, keepdims=True)
            p = e / jnp.where(first, s0, s1)
            return p, block_diag(qkv[:, 2 * PW:3 * PW])

        qkvs, pvs, outs, acc = {}, {}, {}, None
        for t in range(n_pair + LAG3):
            if t < n_pair:
                qkvs[t] = project(t)
            if 0 <= t - LAG1 < n_pair:
                pvs[t - LAG1] = probs(qkvs.pop(t - LAG1))
            if 0 <= t - LAG2 < n_pair:
                outs[t - LAG2] = _dot(*pvs.pop(t - LAG2))
            if 0 <= t - LAG3 < n_pair:
                y = _dot(outs.pop(t - LAG3), pltpu.bitcast(wo_s[t - LAG3], BF16))
                acc = y if acc is None else acc + y

        g = gate[pl.ds(row0, seg), :]
        g = jnp.concatenate([g] * nt, axis=1)
        out_vm[pl.ds(row0, seg), :] = (g * acc[M:, :] + bmix[pl.ds(row0, seg), :]).astype(BF16)
        out_copy(s).start()
        return acc[0:M, :]

    jax.lax.fori_loop(0, n_seg, a_step, mem0_ref[...].astype(F32))
    pltpu.make_async_copy(out_vm, out_hbm, out_sem.at[0]).wait()


@functools.partial(jax.jit, static_argnames=("A_seg_len",))
def pallas_gated_mix__memory_aug_recurrent_mem_tr__sliding_local_dilated__prompt_kernel(
    A_x: jax.Array,
    A_mem0: jax.Array,
    A_Wq: jax.Array,
    A_Wk: jax.Array,
    A_Wv: jax.Array,
    A_Wo: jax.Array,
    A_seg_len: int,
    B_x: jax.Array,
    B_wqkv: jax.Array,
    B_wo: jax.Array,
    gate_w: jax.Array,
):
    del B_x
    _, S, D = A_x.shape
    _, H, dh = A_Wq.shape
    M = A_mem0.shape[1]
    PW = 2 * dh
    n_pair = H // 2

    def rows(w):
        return jnp.transpose(w, (1, 2, 0)).reshape(H * dh, D)

    hbm = pl.BlockSpec(memory_space=pl.ANY)
    vmem = pl.BlockSpec(memory_space=pltpu.VMEM)
    kv_rows = max(HALO + RB, D)
    out = pl.pallas_call(
        functools.partial(_kernel, seg=int(A_seg_len), dh=dh),
        out_shape=jax.ShapeDtypeStruct((S, D), A_x.dtype),
        in_specs=[hbm, vmem, hbm, hbm, hbm, hbm, hbm, hbm, vmem],
        out_specs=hbm,
        scratch_shapes=[
            pltpu.VMEM((S, D), BF16),
            pltpu.VMEM((D, 3 * D), BF16),
            pltpu.VMEM((D, D), BF16),
            pltpu.VMEM((D, 3 * D), BF16),
            pltpu.VMEM((D, D), BF16),
            pltpu.VMEM((n_pair, 4, PW, D), BF16),
            pltpu.VMEM((n_pair, D // 2, 3 * PW), U32),
            pltpu.VMEM((n_pair, PW // 2, D), U32),
            pltpu.VMEM((RB, D), F32),
            pltpu.VMEM((D // LANES, kv_rows, LANES), F32),
            pltpu.VMEM((D // LANES, HALO + RB, LANES), F32),
            pltpu.VMEM((RB, D), BF16),
            pltpu.VMEM((S, D), F32),
            pltpu.VMEM((S, LANES), F32),
            pltpu.VMEM((S, D), BF16),
            pltpu.SemaphoreType.DMA((3,)),
            pltpu.SemaphoreType.DMA((n_pair, 4)),
            pltpu.SemaphoreType.DMA((1,)),
        ],
        compiler_params=pltpu.CompilerParams(vmem_limit_bytes=110 * 2**20),
    )(A_x.reshape(S, D), A_mem0.reshape(M, D), rows(A_Wq), rows(A_Wk), rows(A_Wv),
      A_Wo.reshape(H * dh, D), B_wqkv, B_wo, gate_w.reshape(1, D))
    return out.reshape(A_x.shape)
```

```python
import functools

import jax
import jax.numpy as jnp
import jax.experimental.pallas as pl
import jax.experimental.pallas.tpu as pltpu

F32 = jnp.float32
BF16 = jnp.bfloat16
U32 = jnp.uint32
NEG = -1000000000.0

B_HEADS = 32
B_WIN = 8
B_DIL = 2
HALO = 16
RB = 256
RH = 64
AHEAD = 1
RS = 16
LANES = 128
LAG1, LAG2, LAG3 = 2, 4, 8


def _iota(shape, dim):
    return jax.lax.broadcasted_iota(jnp.int32, shape, dim)


def _aligned(i, n):
    return i if isinstance(i, int) else pl.multiple_of(i, n)


def _when(cond):
    if isinstance(cond, bool):
        return lambda f: f() if cond else None
    return pl.when(cond)


def _dot(a, b):
    return jnp.dot(a, b, preferred_element_type=F32)


def _dot_nt(a, b):
    return jax.lax.dot_general(a, b, (((1,), (1,)), ((), ())), preferred_element_type=F32)


def _kernel(x_hbm, mem0_ref, wq_hbm, wk_hbm, wv_hbm, wo_hbm, bqkv_hbm, bwo_hbm, gw_ref,
            out_hbm,
            x_vm, bqkv_vm, bwo_vm, perm_s, bqkv_p, bwo_p, stage, wqkv_s, wo_s,
            q_b, k_b, v_b, o_b, bmix, gate, out_vm, in_sem, x_sem, w_sem, out_sem,
            *, seg, dh):
    S, D = x_vm.shape
    M = mem0_ref.shape[0]
    L = M + seg
    n_seg = S // seg
    PW = 2 * dh
    n_pair = wo_hbm.shape[0] // PW
    n_blk = S // RB
    ppb = n_pair // n_blk
    nt = D // LANES
    bdh = D // B_HEADS

    cp_bqkv = [pltpu.make_async_copy(bqkv_hbm.at[:, j * D:(j + 1) * D], bqkv_vm.at[j], in_sem.at[j])
               for j in range(3)]
    cp_bwo = pltpu.make_async_copy(bwo_hbm, bwo_vm, in_sem.at[3])

    def x_copy(i):
        rows = pl.ds(_aligned(i * RB, RB), RB)
        return pltpu.make_async_copy(x_hbm.at[rows, :], x_vm.at[rows, :], x_sem.at[i])

    for c in cp_bqkv + [cp_bwo, x_copy(0)]:
        c.start()

    def w_copies(g):
        rows = pl.ds(_aligned(g * PW, PW), PW)
        return [pltpu.make_async_copy(src.at[rows, :], stage.at[g, j], w_sem.at[g, j])
                for j, src in enumerate((wq_hbm, wk_hbm, wv_hbm, wo_hbm))]

    def start_batch(i):
        @_when(i + 1 < n_blk)
        def _():
            x_copy(i + 1).start()

        for t in range(ppb):
            for c in w_copies(i * ppb + t):
                c.start()

    def permuted_rows(ref):
        return jnp.concatenate(
            [ref[pl.ds(d, B_HEADS, stride=bdh), :] for d in range(bdh)], axis=0)

    for j in range(3):
        cp_bqkv[j].wait()
        if j == 2:
            for i in range(AHEAD):
                start_batch(i)
        words = pltpu.bitcast(bqkv_vm[j], U32)
        for u, r in enumerate(range(0, D // 2, LANES)):
            n = min(LANES, D // 2 - r)
            blk = words[r:r + n, :]
            if n < LANES:
                blk = jnp.concatenate([blk] * (LANES // n), axis=0)
            perm_s[u] = blk.T
            bqkv_p[j, r:r + n, :] = permuted_rows(perm_s.at[u]).T[0:n, :]
    cp_bwo.wait()
    wide = bwo_vm[...].astype(F32)
    for t in range(nt):
        k_b[t, 0:D, :] = wide[:, t * LANES:(t + 1) * LANES]
    for d in range(bdh):
        for t in range(nt):
            bwo_p[d * B_HEADS // 2:(d + 1) * B_HEADS // 2, t * LANES:(t + 1) * LANES] = pltpu.bitcast(
                k_b[t, pl.ds(d, B_HEADS, stride=bdh), :].astype(BF16), U32)

    a_scale = dh ** -0.5
    half = dh - LANES

    def out_copy(s):
        rows = pl.ds(_aligned(s * seg, seg), seg)
        return pltpu.make_async_copy(out_vm.at[rows, :], out_hbm.at[rows, :], out_sem.at[0])

    def block_diag(a):
        lo = _iota((L, LANES), 1) < half
        z = jnp.zeros((L, LANES), F32)
        mid = a[:, LANES:2 * LANES]
        top = jnp.concatenate([a[:, 0:LANES], jnp.where(lo, mid, 0.0), z], axis=1)
        bot = jnp.concatenate([z, jnp.where(lo, 0.0, mid), a[:, 2 * LANES:3 * LANES]], axis=1)
        return jnp.concatenate([top, bot], axis=0).astype(BF16)

    def a_rows(s, mem):
        row0 = _aligned(s * seg, seg)
        return jnp.concatenate([mem, x_vm[pl.ds(row0, seg), :].astype(F32)], axis=0)

    def a_project(h, g):
        return _dot(h, pltpu.bitcast(wqkv_s[g], BF16))

    def a_probs(qkv):
        row = _iota((L, 2 * L), 0)
        col = _iota((L, 2 * L), 1)
        first = col < L
        visible = (row < M) | (row >= jnp.where(first, col, col - L))
        sc = _dot_nt(qkv[:, 0:PW], block_diag(qkv[:, PW:2 * PW])) * a_scale
        sc = jnp.where(visible, sc, NEG)
        m0 = jnp.max(jnp.where(first, sc, -jnp.inf), axis=1, keepdims=True)
        m1 = jnp.max(jnp.where(first, -jnp.inf, sc), axis=1, keepdims=True)
        e = jnp.exp(sc - jnp.where(first, m0, m1))
        s0 = jnp.sum(jnp.where(first, e, 0.0), axis=1, keepdims=True)
        s1 = jnp.sum(jnp.where(first, 0.0, e), axis=1, keepdims=True)
        return e / jnp.where(first, s0, s1), block_diag(qkv[:, 2 * PW:3 * PW])

    def a_out(o, g):
        return _dot(o, pltpu.bitcast(wo_s[g], BF16))

    def a_finish(s, acc):
        rows = pl.ds(_aligned(s * seg, seg), seg)
        g = jnp.concatenate([gate[rows, :]] * nt, axis=1)
        out_vm[rows, :] = (g * acc[M:, :] + bmix[rows, :]).astype(BF16)
        out_copy(s).start()
        return acc[0:M, :]

    gw = gw_ref[...].astype(F32)
    b_scale = bdh ** -0.5
    for t in range(nt):
        v_b[t, 0:HALO, :] = jnp.zeros((HALO, LANES), F32)

    def relayout(g):
        for j in range(3):
            wt = stage[g, j].T
            wqkv_s[g, :, j * PW:(j + 1) * PW] = pltpu.bitcast(wt, U32)
        wo_s[g] = pltpu.bitcast(stage[g, 3], U32)

    def b_project(i, r0):
        xb = x_vm[pl.ds(_aligned(i * RB + r0, RH), RH), :]
        k = _dot(xb, pltpu.bitcast(bqkv_p[1], BF16))
        q_b[r0:r0 + RH, :] = _dot(xb, pltpu.bitcast(bqkv_p[0], BF16)) * b_scale
        v = _dot(xb, pltpu.bitcast(bqkv_p[2], BF16))
        for t in range(nt):
            for buf, val in ((k_b, k), (v_b, v)):
                val = val[:, t * LANES:(t + 1) * LANES]
                buf[t, HALO + r0:HALO + r0 + RH, :] = val
                if r0 == 0:
                    buf[t, 0:HALO, :] = jnp.where(
                        i == 0, jnp.broadcast_to(val[0:1, :], (HALO, LANES)), buf[t, 0:HALO, :])

    def b_attend(i, r0):
        for r in range(r0, r0 + RH, RS):
            base = HALO + r
            qs = [q_b[r:r + RS, t * LANES:(t + 1) * LANES] for t in range(nt)]
            logits = []
            for w in range(B_WIN):
                lo = base - w * B_DIL
                acc = qs[0] * k_b[0, lo:lo + RS, :]
                for t in range(1, nt):
                    acc = acc + qs[t] * k_b[t, lo:lo + RS, :]
                acc = acc + pltpu.roll(acc, 64, 1)
                acc = acc + pltpu.roll(acc, 32, 1)
                if r < w * B_DIL:
                    pos = i * RB + r + _iota((RS, LANES), 0)
                    acc = jnp.where(pos >= w * B_DIL, acc, NEG)
                logits.append(acc)
            mx = functools.reduce(jnp.maximum, logits)
            es = [jnp.exp(l - mx) for l in logits]
            inv = 1.0 / functools.reduce(jnp.add, es)
            ps = [e * inv for e in es]
            for t in range(nt):
                acc = ps[0] * v_b[t, base:base + RS, :]
                for w in range(1, B_WIN):
                    lo = base - w * B_DIL
                    acc = acc + ps[w] * v_b[t, lo:lo + RS, :]
                o_b[r:r + RS, t * LANES:(t + 1) * LANES] = acc.astype(BF16)

    def b_finish(i, r0):
        rows = pl.ds(_aligned(i * RB + r0, RH), RH)
        b = _dot(o_b[r0:r0 + RH, :], pltpu.bitcast(bwo_p[...], BF16))
        z = jnp.sum(x_vm[rows, :].astype(F32) * gw, axis=1, keepdims=True)
        g = 1.0 / (1.0 + jnp.exp(-z))
        gate[rows, :] = jnp.broadcast_to(g, (RH, LANES))
        bmix[rows, :] = (1.0 - g) * b

    def b_block(i, acc, with_b=True, with_a=True):
        if with_b:
            @_when(i + AHEAD < n_blk)
            def _():
                start_batch(i + AHEAD)

            x_copy(i).wait()
        gs = [(i - 1) * ppb + t for t in range(ppb)] if with_a else []
        for g in gs:
            for c in w_copies(g):
                c.wait()
        h = a_rows(0, mem0_ref[...].astype(F32))
        nq = RB // RH
        vals = {}
        for t in range(max(nq + 2, ppb + 4)):
            if with_b and t < nq:
                b_project(i, t * RH)
            if with_b and 0 <= t - 1 < nq:
                b_attend(i, (t - 1) * RH)
            for u, g in enumerate(gs):
                stage_id = t - u
                if stage_id == 0:
                    relayout(g)
                elif stage_id == 1:
                    vals[u] = a_project(h, g)
                elif stage_id == 2:
                    vals[u] = a_probs(vals[u])
                elif stage_id == 3:
                    vals[u] = _dot(*vals[u])
                elif stage_id == 4:
                    acc = acc + a_out(vals[u], g)
            if with_b and 0 <= t - 2 < nq:
                b_finish(i, (t - 2) * RH)
        if with_b:
            for t in range(nt):
                k_b[t, 0:HALO, :] = k_b[t, RB:RB + HALO, :]
                v_b[t, 0:HALO, :] = v_b[t, RB:RB + HALO, :]
        return acc

    acc0 = b_block(0, jnp.zeros((L, D), F32), with_a=False)
    acc0 = jax.lax.fori_loop(1, n_blk, b_block, acc0)
    acc0 = b_block(n_blk, acc0, with_b=False)

    def a_step(s, mem):
        h = a_rows(s, mem)
        qkvs, pvs, outs, acc = {}, {}, {}, None
        for t in range(n_pair + LAG3):
            if t < n_pair:
                qkvs[t] = a_project(h, t)
            if 0 <= t - LAG1 < n_pair:
                pvs[t - LAG1] = a_probs(qkvs.pop(t - LAG1))
            if 0 <= t - LAG2 < n_pair:
                outs[t - LAG2] = _dot(*pvs.pop(t - LAG2))
            if 0 <= t - LAG3 < n_pair:
                y = a_out(outs.pop(t - LAG3), t - LAG3)
                acc = y if acc is None else acc + y
        return a_finish(s, acc)

    jax.lax.fori_loop(1, n_seg, a_step, a_finish(0, acc0))
    pltpu.make_async_copy(out_vm, out_hbm, out_sem.at[0]).wait()


@functools.partial(jax.jit, static_argnames=("A_seg_len",))
def pallas_gated_mix__memory_aug_recurrent_mem_tr__sliding_local_dilated__prompt_kernel(
    A_x: jax.Array,
    A_mem0: jax.Array,
    A_Wq: jax.Array,
    A_Wk: jax.Array,
    A_Wv: jax.Array,
    A_Wo: jax.Array,
    A_seg_len: int,
    B_x: jax.Array,
    B_wqkv: jax.Array,
    B_wo: jax.Array,
    gate_w: jax.Array,
):
    del B_x
    _, S, D = A_x.shape
    _, H, dh = A_Wq.shape
    M = A_mem0.shape[1]
    PW = 2 * dh
    n_pair = H // 2

    def rows(w):
        return jnp.transpose(w, (1, 2, 0)).reshape(H * dh, D)

    hbm = pl.BlockSpec(memory_space=pl.ANY)
    vmem = pl.BlockSpec(memory_space=pltpu.VMEM)
    kv_rows = max(HALO + RB, D)
    out = pl.pallas_call(
        functools.partial(_kernel, seg=int(A_seg_len), dh=dh),
        out_shape=jax.ShapeDtypeStruct((S, D), A_x.dtype),
        in_specs=[hbm, vmem, hbm, hbm, hbm, hbm, hbm, hbm, vmem],
        out_specs=hbm,
        scratch_shapes=[
            pltpu.VMEM((S, D), BF16),
            pltpu.VMEM((3, D, D), BF16),
            pltpu.VMEM((D, D), BF16),
            pltpu.VMEM((pl.cdiv(D // 2, LANES), D, LANES), U32),
            pltpu.VMEM((3, D // 2, D), U32),
            pltpu.VMEM((D // 2, D), U32),
            pltpu.VMEM((n_pair, 4, PW, D), BF16),
            pltpu.VMEM((n_pair, D // 2, 3 * PW), U32),
            pltpu.VMEM((n_pair, PW // 2, D), U32),
            pltpu.VMEM((RB, D), F32),
            pltpu.VMEM((D // LANES, kv_rows, LANES), F32),
            pltpu.VMEM((D // LANES, HALO + RB, LANES), F32),
            pltpu.VMEM((RB, D), BF16),
            pltpu.VMEM((S, D), F32),
            pltpu.VMEM((S, LANES), F32),
            pltpu.VMEM((S, D), BF16),
            pltpu.SemaphoreType.DMA((4,)),
            pltpu.SemaphoreType.DMA((S // RB,)),
            pltpu.SemaphoreType.DMA((n_pair, 4)),
            pltpu.SemaphoreType.DMA((1,)),
        ],
        compiler_params=pltpu.CompilerParams(vmem_limit_bytes=110 * 2**20),
    )(A_x.reshape(S, D), A_mem0.reshape(M, D), rows(A_Wq), rows(A_Wk), rows(A_Wv),
      A_Wo.reshape(H * dh, D), B_wqkv, B_wo, gate_w.reshape(1, D))
    return out.reshape(A_x.shape)
```

```python
import functools

import jax
import jax.numpy as jnp
import jax.experimental.pallas as pl
import jax.experimental.pallas.tpu as pltpu

F32 = jnp.float32
BF16 = jnp.bfloat16
U32 = jnp.uint32
NEG = -1000000000.0

B_HEADS = 32
B_WIN = 8
B_DIL = 2
HALO = 16
RB = 256
RH = 128
AHEAD = 1
RS = 16
LANES = 128
LAG1, LAG2, LAG3 = 2, 4, 8
TAIL = 4
UNROLL = 3


def _iota(shape, dim):
    return jax.lax.broadcasted_iota(jnp.int32, shape, dim)


def _aligned(i, n):
    return i if isinstance(i, int) else pl.multiple_of(i, n)


def _when(cond):
    if isinstance(cond, bool):
        return lambda f: f() if cond else None
    return pl.when(cond)


def _dot(a, b):
    return jnp.dot(a, b, preferred_element_type=F32)


def _dot_nt(a, b):
    return jax.lax.dot_general(a, b, (((1,), (1,)), ((), ())), preferred_element_type=F32)


def _kernel(x_hbm, mem0_ref, wq_hbm, wk_hbm, wv_hbm, wo_hbm, bqkv_hbm, bwo_hbm, gw_ref,
            out_hbm,
            x_vm, bqkv_vm, bwo_vm, perm_s, bqkv_p, bwo_p, stage, wqkv_s, wo_s,
            q_b, k_b, v_b, o_b, bmix, gate, out_vm, in_sem, x_sem, w_sem, out_sem,
            *, seg, dh):
    S, D = x_vm.shape
    M = mem0_ref.shape[0]
    L = M + seg
    n_seg = S // seg
    PW = 2 * dh
    n_pair = wo_hbm.shape[0] // PW
    n_blk = S // RB
    ppb = n_pair // n_blk
    nt = D // LANES
    bdh = D // B_HEADS

    cp_bqkv = [pltpu.make_async_copy(bqkv_hbm.at[:, j * D:(j + 1) * D], bqkv_vm.at[j], in_sem.at[j])
               for j in range(3)]
    cp_bwo = pltpu.make_async_copy(bwo_hbm, bwo_vm, in_sem.at[3])

    def x_copy(i):
        rows = pl.ds(_aligned(i * RB, RB), RB)
        return pltpu.make_async_copy(x_hbm.at[rows, :], x_vm.at[rows, :], x_sem.at[i])

    for c in cp_bqkv + [cp_bwo, x_copy(0)]:
        c.start()

    def w_copies(g):
        rows = pl.ds(_aligned(g * PW, PW), PW)
        return [pltpu.make_async_copy(src.at[rows, :], stage.at[g, j], w_sem.at[g, j])
                for j, src in enumerate((wq_hbm, wk_hbm, wv_hbm, wo_hbm))]

    def start_batch(i):
        @_when(i + 1 < n_blk)
        def _():
            x_copy(i + 1).start()

        for t in range(ppb):
            for c in w_copies(i * ppb + t):
                c.start()

    def permuted_rows(ref):
        return jnp.concatenate(
            [ref[pl.ds(d, B_HEADS, stride=bdh), :] for d in range(bdh)], axis=0)

    for j in range(3):
        cp_bqkv[j].wait()
        if j == 2:
            for i in range(AHEAD):
                start_batch(i)
        words = pltpu.bitcast(bqkv_vm[j], U32)
        for u, r in enumerate(range(0, D // 2, LANES)):
            n = min(LANES, D // 2 - r)
            blk = words[r:r + n, :]
            if n < LANES:
                blk = jnp.concatenate([blk] * (LANES // n), axis=0)
            perm_s[u] = blk.T
            bqkv_p[j, r:r + n, :] = permuted_rows(perm_s.at[u]).T[0:n, :]
    cp_bwo.wait()
    wide = bwo_vm[...].astype(F32)
    for t in range(nt):
        k_b[t, 0:D, :] = wide[:, t * LANES:(t + 1) * LANES]
    for d in range(bdh):
        for t in range(nt):
            bwo_p[d * B_HEADS // 2:(d + 1) * B_HEADS // 2, t * LANES:(t + 1) * LANES] = pltpu.bitcast(
                k_b[t, pl.ds(d, B_HEADS, stride=bdh), :].astype(BF16), U32)

    a_scale = dh ** -0.5
    half = dh - LANES

    def out_copy(s):
        rows = pl.ds(_aligned(s * seg, seg), seg)
        return pltpu.make_async_copy(out_vm.at[rows, :], out_hbm.at[rows, :], out_sem.at[0])

    def block_diag(a):
        lo = _iota((L, LANES), 1) < half
        z = jnp.zeros((L, LANES), F32)
        mid = a[:, LANES:2 * LANES]
        top = jnp.concatenate([a[:, 0:LANES], jnp.where(lo, mid, 0.0), z], axis=1)
        bot = jnp.concatenate([z, jnp.where(lo, 0.0, mid), a[:, 2 * LANES:3 * LANES]], axis=1)
        return jnp.concatenate([top, bot], axis=0).astype(BF16)

    def a_rows(s, mem):
        row0 = _aligned(s * seg, seg)
        return jnp.concatenate([mem, x_vm[pl.ds(row0, seg), :].astype(F32)], axis=0)

    def a_project(h, g):
        return _dot(h, pltpu.bitcast(wqkv_s[g], BF16))

    def a_probs(qkv):
        row = _iota((L, 2 * L), 0)
        col = _iota((L, 2 * L), 1)
        first = col < L
        visible = (row < M) | (row >= jnp.where(first, col, col - L))
        sc = _dot_nt(qkv[:, 0:PW], block_diag(qkv[:, PW:2 * PW])) * a_scale
        sc = jnp.where(visible, sc, NEG)
        m0 = jnp.max(jnp.where(first, sc, -jnp.inf), axis=1, keepdims=True)
        m1 = jnp.max(jnp.where(first, -jnp.inf, sc), axis=1, keepdims=True)
        e = jnp.exp(sc - jnp.where(first, m0, m1))
        s0 = jnp.sum(jnp.where(first, e, 0.0), axis=1, keepdims=True)
        s1 = jnp.sum(jnp.where(first, 0.0, e), axis=1, keepdims=True)
        return e / jnp.where(first, s0, s1), block_diag(qkv[:, 2 * PW:3 * PW])

    def a_out(o, g):
        return _dot(o, pltpu.bitcast(wo_s[g], BF16))

    def a_finish(s, acc):
        rows = pl.ds(_aligned(s * seg, seg), seg)
        g = jnp.concatenate([gate[rows, :]] * nt, axis=1)
        out_vm[rows, :] = (g * acc[M:, :] + bmix[rows, :]).astype(BF16)
        out_copy(s).start()
        return acc[0:M, :]

    gw = gw_ref[...].astype(F32)
    b_scale = bdh ** -0.5
    for t in range(nt):
        v_b[t, 0:HALO, :] = jnp.zeros((HALO, LANES), F32)

    def relayout(g):
        for j in range(3):
            wt = stage[g, j].T
            wqkv_s[g, :, j * PW:(j + 1) * PW] = pltpu.bitcast(wt, U32)
        wo_s[g] = pltpu.bitcast(stage[g, 3], U32)

    def b_project(i, r0):
        xb = x_vm[pl.ds(_aligned(i * RB + r0, RH), RH), :]
        k = _dot(xb, pltpu.bitcast(bqkv_p[1], BF16))
        q_b[r0:r0 + RH, :] = _dot(xb, pltpu.bitcast(bqkv_p[0], BF16)) * b_scale
        v = _dot(xb, pltpu.bitcast(bqkv_p[2], BF16))
        for t in range(nt):
            for buf, val in ((k_b, k), (v_b, v)):
                val = val[:, t * LANES:(t + 1) * LANES]
                buf[t, HALO + r0:HALO + r0 + RH, :] = val
                if r0 == 0:
                    buf[t, 0:HALO, :] = jnp.where(
                        i == 0, jnp.broadcast_to(val[0:1, :], (HALO, LANES)), buf[t, 0:HALO, :])

    def b_attend(i, r0):
        for r in range(r0, r0 + RH, RS):
            base = HALO + r
            qs = [q_b[r:r + RS, t * LANES:(t + 1) * LANES] for t in range(nt)]
            logits = []
            for w in range(B_WIN):
                lo = base - w * B_DIL
                acc = qs[0] * k_b[0, lo:lo + RS, :]
                for t in range(1, nt):
                    acc = acc + qs[t] * k_b[t, lo:lo + RS, :]
                acc = acc + pltpu.roll(acc, 64, 1)
                acc = acc + pltpu.roll(acc, 32, 1)
                if r < w * B_DIL:
                    pos = i * RB + r + _iota((RS, LANES), 0)
                    acc = jnp.where(pos >= w * B_DIL, acc, NEG)
                logits.append(acc)
            mx = functools.reduce(jnp.maximum, logits)
            es = [jnp.exp(l - mx) for l in logits]
            inv = 1.0 / functools.reduce(jnp.add, es)
            ps = [e * inv for e in es]
            for t in range(nt):
                acc = ps[0] * v_b[t, base:base + RS, :]
                for w in range(1, B_WIN):
                    lo = base - w * B_DIL
                    acc = acc + ps[w] * v_b[t, lo:lo + RS, :]
                o_b[r:r + RS, t * LANES:(t + 1) * LANES] = acc.astype(BF16)

    def b_finish(i, r0):
        rows = pl.ds(_aligned(i * RB + r0, RH), RH)
        b = _dot(o_b[r0:r0 + RH, :], pltpu.bitcast(bwo_p[...], BF16))
        z = jnp.sum(x_vm[rows, :].astype(F32) * gw, axis=1, keepdims=True)
        g = 1.0 / (1.0 + jnp.exp(-z))
        gate[rows, :] = jnp.broadcast_to(g, (RH, LANES))
        bmix[rows, :] = (1.0 - g) * b

    def b_block(i, acc, with_b=True, with_a=True):
        gs = [(i - 1) * ppb + t for t in range(ppb)] if with_a else []
        for g in gs:
            for c in w_copies(g):
                c.wait()
        if with_b:
            x_copy(i).wait()

            @_when(i + AHEAD < n_blk)
            def _():
                start_batch(i + AHEAD)

        h = a_rows(0, mem0_ref[...].astype(F32))
        nq = RB // RH
        vals = {}
        for t in range(max(nq + 2, ppb + 4)):
            if with_b and t < nq:
                b_project(i, t * RH)
            if with_b and 0 <= t - 1 < nq:
                b_attend(i, (t - 1) * RH)
            for u, g in enumerate(gs):
                stage_id = t - u
                if stage_id == 0:
                    relayout(g)
                elif stage_id == 1:
                    vals[u] = a_project(h, g)
                elif stage_id == 2:
                    vals[u] = a_probs(vals[u])
                elif stage_id == 3:
                    vals[u] = _dot(*vals[u])
                elif stage_id == 4:
                    acc = acc + a_out(vals[u], g)
            if with_b and 0 <= t - 2 < nq:
                b_finish(i, (t - 2) * RH)
        if with_b:
            for t in range(nt):
                k_b[t, 0:HALO, :] = k_b[t, RB:RB + HALO, :]
                v_b[t, 0:HALO, :] = v_b[t, RB:RB + HALO, :]
        return acc

    acc0 = b_block(0, jnp.zeros((L, D), F32), with_a=False)
    acc0 = jax.lax.fori_loop(1, n_blk, b_block, acc0)
    acc0 = b_block(n_blk, acc0, with_b=False)

    def a_step(s, mem):
        h = a_rows(s, mem)
        qkvs, pvs, outs, acc = {}, {}, {}, None
        for t in range(n_pair + LAG2):
            if t == 0:
                qkvs[t] = functools.reduce(jnp.add, [
                    _dot(h[:, c * LANES:(c + 1) * LANES],
                         pltpu.bitcast(wqkv_s[t, c * LANES // 2:(c + 1) * LANES // 2, :], BF16))
                    for c in range(nt)])
            elif t < n_pair:
                qkvs[t] = a_project(h, t)
            if 0 <= t - LAG1 < n_pair:
                pvs[t - LAG1] = a_probs(qkvs.pop(t - LAG1))
            if 0 <= t - LAG2 < n_pair:
                outs[t - LAG2] = _dot(*pvs.pop(t - LAG2))
            g = t - LAG3
            if t >= n_pair:
                g = n_pair - LAG3 + (t - n_pair)
            if 0 <= g < n_pair - TAIL:
                y = a_out(outs.pop(g), g)
                acc = y if acc is None else acc + y
        left = sorted(outs)
        o = jnp.concatenate([outs[g] for g in left], axis=1)
        cols = []
        for c in range(nt):
            w = wo_s[left[0]:n_pair, :, c * LANES:(c + 1) * LANES].reshape(-1, LANES)
            cols.append(acc[:, c * LANES:(c + 1) * LANES] + _dot(o, pltpu.bitcast(w, BF16)))
        return a_finish(s, jnp.concatenate(cols, axis=1))

    def a_steps(i, mem):
        for u in range(UNROLL):
            mem = a_step(1 + i * UNROLL + u, mem)
        return mem

    assert (n_seg - 1) % UNROLL == 0
    jax.lax.fori_loop(0, (n_seg - 1) // UNROLL, a_steps, a_finish(0, acc0))
    pltpu.make_async_copy(out_vm, out_hbm, out_sem.at[0]).wait()


@functools.partial(jax.jit, static_argnames=("A_seg_len",))
def pallas_gated_mix__memory_aug_recurrent_mem_tr__sliding_local_dilated__prompt_kernel(
    A_x: jax.Array,
    A_mem0: jax.Array,
    A_Wq: jax.Array,
    A_Wk: jax.Array,
    A_Wv: jax.Array,
    A_Wo: jax.Array,
    A_seg_len: int,
    B_x: jax.Array,
    B_wqkv: jax.Array,
    B_wo: jax.Array,
    gate_w: jax.Array,
):
    del B_x
    _, S, D = A_x.shape
    _, H, dh = A_Wq.shape
    M = A_mem0.shape[1]
    PW = 2 * dh
    n_pair = H // 2

    def rows(w):
        return jnp.transpose(w, (1, 2, 0)).reshape(H * dh, D)

    hbm = pl.BlockSpec(memory_space=pl.ANY)
    vmem = pl.BlockSpec(memory_space=pltpu.VMEM)
    kv_rows = max(HALO + RB, D)
    out = pl.pallas_call(
        functools.partial(_kernel, seg=int(A_seg_len), dh=dh),
        out_shape=jax.ShapeDtypeStruct((S, D), A_x.dtype),
        in_specs=[hbm, vmem, hbm, hbm, hbm, hbm, hbm, hbm, vmem],
        out_specs=hbm,
        scratch_shapes=[
            pltpu.VMEM((S, D), BF16),
            pltpu.VMEM((3, D, D), BF16),
            pltpu.VMEM((D, D), BF16),
            pltpu.VMEM((pl.cdiv(D // 2, LANES), D, LANES), U32),
            pltpu.VMEM((3, D // 2, D), U32),
            pltpu.VMEM((D // 2, D), U32),
            pltpu.VMEM((n_pair, 4, PW, D), BF16),
            pltpu.VMEM((n_pair, D // 2, 3 * PW), U32),
            pltpu.VMEM((n_pair, PW // 2, D), U32),
            pltpu.VMEM((RB, D), F32),
            pltpu.VMEM((D // LANES, kv_rows, LANES), F32),
            pltpu.VMEM((D // LANES, HALO + RB, LANES), F32),
            pltpu.VMEM((RB, D), BF16),
            pltpu.VMEM((S, D), F32),
            pltpu.VMEM((S, LANES), F32),
            pltpu.VMEM((S, D), BF16),
            pltpu.SemaphoreType.DMA((4,)),
            pltpu.SemaphoreType.DMA((S // RB,)),
            pltpu.SemaphoreType.DMA((n_pair, 4)),
            pltpu.SemaphoreType.DMA((1,)),
        ],
        compiler_params=pltpu.CompilerParams(vmem_limit_bytes=110 * 2**20),
    )(A_x.reshape(S, D), A_mem0.reshape(M, D), rows(A_Wq), rows(A_Wk), rows(A_Wv),
      A_Wo.reshape(H * dh, D), B_wqkv, B_wo, gate_w.reshape(1, D))
    return out.reshape(A_x.shape)
```

```python
import functools

import jax
import jax.numpy as jnp
import jax.experimental.pallas as pl
import jax.experimental.pallas.tpu as pltpu

F32 = jnp.float32
BF16 = jnp.bfloat16
U32 = jnp.uint32
NEG = -1000000000.0

B_HEADS = 32
B_WIN = 8
B_DIL = 2
HALO = 16
RB = 256
RH = 128
AHEAD = 1
RS = 16
LANES = 128
LAG1, LAG2, LAG3 = 1, 4, 8
TAIL = 4
UNROLL = 3


def _iota(shape, dim):
    return jax.lax.broadcasted_iota(jnp.int32, shape, dim)


def _aligned(i, n):
    return i if isinstance(i, int) else pl.multiple_of(i, n)


def _when(cond):
    if isinstance(cond, bool):
        return lambda f: f() if cond else None
    return pl.when(cond)


def _dot(a, b):
    return jnp.dot(a, b, preferred_element_type=F32)


def _dot_nt(a, b):
    return jax.lax.dot_general(a, b, (((1,), (1,)), ((), ())), preferred_element_type=F32)


def _kernel(x_hbm, mem0_ref, wq_hbm, wk_hbm, wv_hbm, wo_hbm, bqkv_hbm, bwo_hbm, gw_ref,
            out_hbm,
            x_vm, bqkv_vm, bwo_vm, perm_s, bwo_t, bqkv_p, bwo_p, stage, wqkv_s, wo_s,
            q_b, k_b, v_b, o_b, bmix, gate, out_vm, in_sem, x_sem, w_sem, out_sem,
            *, seg, dh):
    S, D = x_vm.shape
    M = mem0_ref.shape[0]
    L = M + seg
    n_seg = S // seg
    PW = 2 * dh
    n_pair = wo_hbm.shape[0] // PW
    n_blk = S // RB
    ppb = n_pair // n_blk
    nt = D // LANES
    bdh = D // B_HEADS

    cp_bqkv = [pltpu.make_async_copy(bqkv_hbm.at[:, j * D:(j + 1) * D], bqkv_vm.at[j], in_sem.at[j])
               for j in range(3)]
    cp_bwo = pltpu.make_async_copy(bwo_hbm, bwo_vm, in_sem.at[3])

    def x_copy(i):
        rows = pl.ds(_aligned(i * RB, RB), RB)
        return pltpu.make_async_copy(x_hbm.at[rows, :], x_vm.at[rows, :], x_sem.at[i])

    for c in (cp_bqkv[1], cp_bqkv[0], cp_bqkv[2], cp_bwo, x_copy(0)):
        c.start()

    def w_copies(g):
        rows = pl.ds(_aligned(g * (PW // 2), PW // 2), PW // 2)
        dsts = [stage.at[g, 0], stage.at[g, 1], stage.at[g, 2], wo_s.at[g]]
        return [pltpu.make_async_copy(src.bitcast(U32).at[rows, :], dsts[j], w_sem.at[g, j])
                for j, src in enumerate((wq_hbm, wk_hbm, wv_hbm, wo_hbm))]

    def start_batch(i):
        @_when(i + 1 < n_blk)
        def _():
            x_copy(i + 1).start()

        for t in range(ppb):
            for c in w_copies(i * ppb + t):
                c.start()

    def permuted_rows(ref):
        return jnp.concatenate(
            [ref[pl.ds(d, B_HEADS, stride=bdh), :] for d in range(bdh)], axis=0)

    for j in (1, 0, 2):
        if j == 1:
            cp_bqkv[1].wait()
        elif j == 0:
            for c in (cp_bqkv[0], cp_bqkv[2], cp_bwo, x_copy(0)):
                c.wait()
            for i in range(AHEAD + 1):
                start_batch(i)
        words = pltpu.bitcast(bqkv_vm[j], U32)
        for u, r in enumerate(range(0, D // 2, LANES)):
            n = min(LANES, D // 2 - r)
            blk = words[r:r + n, :]
            if n < LANES:
                blk = jnp.concatenate([blk] * (LANES // n), axis=0)
            perm_s[j, u] = blk.T
            bqkv_p[j, r:r + n, :] = permuted_rows(perm_s.at[j, u]).T[0:n, :]
    for t in range(nt):
        bwo_t[t] = bwo_vm[:, t * LANES:(t + 1) * LANES].astype(F32)
        bwo_p[:, t * LANES:(t + 1) * LANES] = pltpu.bitcast(
            permuted_rows(bwo_t.at[t]).astype(BF16), U32)

    a_scale = dh ** -0.5
    half = dh - LANES

    def out_copy(s):
        rows = pl.ds(_aligned(s * seg, seg), seg)
        return pltpu.make_async_copy(out_vm.at[rows, :], out_hbm.at[rows, :], out_sem.at[0])

    def block_diag(a):
        lo = _iota((L, LANES), 1) < half
        z = jnp.zeros((L, LANES), F32)
        mid = a[:, LANES:2 * LANES]
        top = jnp.concatenate([a[:, 0:LANES], jnp.where(lo, mid, 0.0), z], axis=1)
        bot = jnp.concatenate([z, jnp.where(lo, 0.0, mid), a[:, 2 * LANES:3 * LANES]], axis=1)
        return jnp.concatenate([top, bot], axis=0).astype(BF16)

    def a_rows(s, mem):
        row0 = _aligned(s * seg, seg)
        return jnp.concatenate([mem, x_vm[pl.ds(row0, seg), :].astype(F32)], axis=0)

    def a_project(h, g):
        return _dot(h, pltpu.bitcast(wqkv_s[g], BF16))

    def a_probs(qkv):
        row = _iota((L, 2 * L), 0)
        col = _iota((L, 2 * L), 1)
        first = col < L
        visible = (row < M) | (row >= jnp.where(first, col, col - L))
        sc = _dot_nt(qkv[:, 0:PW], block_diag(qkv[:, PW:2 * PW])) * a_scale
        sc = jnp.where(visible, sc, NEG)
        m0 = jnp.max(jnp.where(first, sc, -jnp.inf), axis=1, keepdims=True)
        m1 = jnp.max(jnp.where(first, -jnp.inf, sc), axis=1, keepdims=True)
        e = jnp.exp(sc - jnp.where(first, m0, m1))
        s0 = jnp.sum(jnp.where(first, e, 0.0), axis=1, keepdims=True)
        s1 = jnp.sum(jnp.where(first, 0.0, e), axis=1, keepdims=True)
        return e / jnp.where(first, s0, s1), block_diag(qkv[:, 2 * PW:3 * PW])

    def a_out(o, g):
        return _dot(o, pltpu.bitcast(wo_s[g], BF16))

    def a_finish(s, acc):
        rows = pl.ds(_aligned(s * seg, seg), seg)
        g = jnp.concatenate([gate[rows, :]] * nt, axis=1)
        out_vm[rows, :] = (g * acc[M:, :] + bmix[rows, :]).astype(BF16)
        out_copy(s).start()
        return acc[0:M, :]

    gw = gw_ref[...].astype(F32)
    b_scale = bdh ** -0.5
    for t in range(nt):
        k_b[t, 0:HALO, :] = jnp.zeros((HALO, LANES), F32)
        v_b[t, 0:HALO, :] = jnp.zeros((HALO, LANES), F32)

    def relayout(g):
        for j in range(3):
            wt = pltpu.bitcast(stage[g, j], BF16).T
            wqkv_s[g, :, j * PW:(j + 1) * PW] = pltpu.bitcast(wt, U32)

    def b_project(i, r0):
        xb = x_vm[pl.ds(_aligned(i * RB + r0, RH), RH), :]
        k = _dot(xb, pltpu.bitcast(bqkv_p[1], BF16))
        q_b[r0:r0 + RH, :] = _dot(xb, pltpu.bitcast(bqkv_p[0], BF16)) * b_scale
        v = _dot(xb, pltpu.bitcast(bqkv_p[2], BF16))
        for t in range(nt):
            for buf, val in ((k_b, k), (v_b, v)):
                val = val[:, t * LANES:(t + 1) * LANES]
                buf[t, HALO + r0:HALO + r0 + RH, :] = val
                if r0 == 0:
                    buf[t, 0:HALO, :] = jnp.where(
                        i == 0, jnp.broadcast_to(val[0:1, :], (HALO, LANES)), buf[t, 0:HALO, :])

    def b_attend(i, r0):
        for r in range(r0, r0 + RH, RS):
            base = HALO + r
            qs = [q_b[r:r + RS, t * LANES:(t + 1) * LANES] for t in range(nt)]
            logits = []
            for w in range(B_WIN):
                lo = base - w * B_DIL
                acc = qs[0] * k_b[0, lo:lo + RS, :]
                for t in range(1, nt):
                    acc = acc + qs[t] * k_b[t, lo:lo + RS, :]
                acc = acc + pltpu.roll(acc, 64, 1)
                acc = acc + pltpu.roll(acc, 32, 1)
                if r < w * B_DIL:
                    pos = i * RB + r + _iota((RS, LANES), 0)
                    acc = jnp.where(pos >= w * B_DIL, acc, NEG)
                logits.append(acc)
            mx = functools.reduce(jnp.maximum, logits)
            es = [jnp.exp(l - mx) for l in logits]
            inv = 1.0 / functools.reduce(jnp.add, es)
            ps = [e * inv for e in es]
            for t in range(nt):
                acc = ps[0] * v_b[t, base:base + RS, :]
                for w in range(1, B_WIN):
                    lo = base - w * B_DIL
                    acc = acc + ps[w] * v_b[t, lo:lo + RS, :]
                o_b[r:r + RS, t * LANES:(t + 1) * LANES] = acc.astype(BF16)

    def b_finish(i, r0):
        rows = pl.ds(_aligned(i * RB + r0, RH), RH)
        b = _dot(o_b[r0:r0 + RH, :], pltpu.bitcast(bwo_p[...], BF16))
        z = jnp.sum(x_vm[rows, :].astype(F32) * gw, axis=1, keepdims=True)
        g = 1.0 / (1.0 + jnp.exp(-z))
        gate[rows, :] = jnp.broadcast_to(g, (RH, LANES))
        bmix[rows, :] = (1.0 - g) * b

    def b_block(i, acc, with_b=True, with_a=True):
        gs = [(i - 1) * ppb + t for t in range(ppb)] if with_a else []
        for g in gs:
            for c in w_copies(g):
                c.wait()
        if with_b and with_a:
            x_copy(i).wait()

            @_when(i + AHEAD < n_blk)
            def _():
                start_batch(i + AHEAD)

        h = a_rows(0, mem0_ref[...].astype(F32))
        nq = RB // RH
        vals = {}
        for t in range(max(nq + 2, ppb + 4)):
            if with_b and t < nq:
                b_project(i, t * RH)
            if with_b and 0 <= t - 1 < nq:
                b_attend(i, (t - 1) * RH)
            for u, g in enumerate(gs):
                stage_id = t - u
                if stage_id == 0:
                    relayout(g)
                elif stage_id == 1:
                    vals[u] = a_project(h, g)
                elif stage_id == 2:
                    vals[u] = a_probs(vals[u])
                elif stage_id == 3:
                    vals[u] = _dot(*vals[u])
                elif stage_id == 4:
                    acc = acc + a_out(vals[u], g)
            if with_b and 0 <= t - 2 < nq:
                b_finish(i, (t - 2) * RH)
        if with_b:
            for t in range(nt):
                k_b[t, 0:HALO, :] = k_b[t, RB:RB + HALO, :]
                v_b[t, 0:HALO, :] = v_b[t, RB:RB + HALO, :]
        return acc

    acc0 = b_block(0, jnp.zeros((L, D), F32), with_a=False)
    acc0 = jax.lax.fori_loop(1, n_blk, b_block, acc0)
    acc0 = b_block(n_blk, acc0, with_b=False)

    def a_step(s, mem):
        h = a_rows(s, mem)
        qkvs, pvs, outs, acc = {}, {}, {}, None
        for t in range(n_pair + LAG2):
            if t == 0:
                qkvs[t] = functools.reduce(jnp.add, [
                    _dot(h[:, c * LANES:(c + 1) * LANES],
                         pltpu.bitcast(wqkv_s[t, c * LANES // 2:(c + 1) * LANES // 2, :], BF16))
                    for c in range(nt)])
            elif t < n_pair:
                qkvs[t] = a_project(h, t)
            if 0 <= t - LAG1 < n_pair:
                pvs[t - LAG1] = a_probs(qkvs.pop(t - LAG1))
            if 0 <= t - LAG2 < n_pair:
                outs[t - LAG2] = _dot(*pvs.pop(t - LAG2))
            g = t - LAG3
            if t >= n_pair:
                g = n_pair - LAG3 + (t - n_pair)
            if 0 <= g < n_pair - TAIL:
                y = a_out(outs.pop(g), g)
                acc = y if acc is None else acc + y
        left = sorted(outs)
        o = jnp.concatenate([outs[g] for g in left], axis=1)
        cols = []
        for c in range(nt):
            w = wo_s[left[0]:n_pair, :, c * LANES:(c + 1) * LANES].reshape(-1, LANES)
            cols.append(acc[:, c * LANES:(c + 1) * LANES] + _dot(o, pltpu.bitcast(w, BF16)))
        return a_finish(s, jnp.concatenate(cols, axis=1))

    def a_steps(i, mem):
        for u in range(UNROLL):
            mem = a_step(1 + i * UNROLL + u, mem)
        return mem

    assert (n_seg - 1) % UNROLL == 0
    jax.lax.fori_loop(0, (n_seg - 1) // UNROLL, a_steps, a_finish(0, acc0))
    pltpu.make_async_copy(out_vm, out_hbm, out_sem.at[0]).wait()


@functools.partial(jax.jit, static_argnames=("A_seg_len",))
def pallas_gated_mix__memory_aug_recurrent_mem_tr__sliding_local_dilated__prompt_kernel(
    A_x: jax.Array,
    A_mem0: jax.Array,
    A_Wq: jax.Array,
    A_Wk: jax.Array,
    A_Wv: jax.Array,
    A_Wo: jax.Array,
    A_seg_len: int,
    B_x: jax.Array,
    B_wqkv: jax.Array,
    B_wo: jax.Array,
    gate_w: jax.Array,
):
    del B_x
    _, S, D = A_x.shape
    _, H, dh = A_Wq.shape
    M = A_mem0.shape[1]
    PW = 2 * dh
    n_pair = H // 2

    def rows(w):
        return jnp.transpose(w, (1, 2, 0)).reshape(H * dh, D)

    hbm = pl.BlockSpec(memory_space=pl.ANY)
    vmem = pl.BlockSpec(memory_space=pltpu.VMEM)
    out = pl.pallas_call(
        functools.partial(_kernel, seg=int(A_seg_len), dh=dh),
        out_shape=jax.ShapeDtypeStruct((S, D), A_x.dtype),
        in_specs=[hbm, vmem, hbm, hbm, hbm, hbm, hbm, hbm, vmem],
        out_specs=hbm,
        scratch_shapes=[
            pltpu.VMEM((S, D), BF16),
            pltpu.VMEM((3, D, D), BF16),
            pltpu.VMEM((D, D), BF16),
            pltpu.VMEM((3, pl.cdiv(D // 2, LANES), D, LANES), U32),
            pltpu.VMEM((D // LANES, D, LANES), F32),
            pltpu.VMEM((3, D // 2, D), U32),
            pltpu.VMEM((D // 2, D), U32),
            pltpu.VMEM((n_pair, 3, PW // 2, D), U32),
            pltpu.VMEM((n_pair, D // 2, 3 * PW), U32),
            pltpu.VMEM((n_pair, PW // 2, D), U32),
            pltpu.VMEM((RB, D), F32),
            pltpu.VMEM((D // LANES, HALO + RB, LANES), F32),
            pltpu.VMEM((D // LANES, HALO + RB, LANES), F32),
            pltpu.VMEM((RB, D), BF16),
            pltpu.VMEM((S, D), F32),
            pltpu.VMEM((S, LANES), F32),
            pltpu.VMEM((S, D), BF16),
            pltpu.SemaphoreType.DMA((4,)),
            pltpu.SemaphoreType.DMA((S // RB,)),
            pltpu.SemaphoreType.DMA((n_pair, 4)),
            pltpu.SemaphoreType.DMA((1,)),
        ],
        compiler_params=pltpu.CompilerParams(vmem_limit_bytes=110 * 2**20),
    )(A_x.reshape(S, D), A_mem0.reshape(M, D), rows(A_Wq), rows(A_Wk), rows(A_Wv),
      A_Wo.reshape(H * dh, D), B_wqkv, B_wo, gate_w.reshape(1, D))
    return out.reshape(A_x.shape)
```

```python
import functools

import jax
import jax.numpy as jnp
import jax.experimental.pallas as pl
import jax.experimental.pallas.tpu as pltpu

F32 = jnp.float32
BF16 = jnp.bfloat16
U32 = jnp.uint32
NEG = -1000000000.0

B_HEADS = 32
B_WIN = 8
B_DIL = 2
HALO = 16
RB = 256
RH = 128
RS = 16
LANES = 128
LAG1, LAG2, LAG3 = 1, 4, 8
TAIL = 4
UNROLL = 3


def _iota(shape, dim):
    return jax.lax.broadcasted_iota(jnp.int32, shape, dim)


def _aligned(i, n):
    return i if isinstance(i, int) else pl.multiple_of(i, n)


def _when(cond):
    if isinstance(cond, bool):
        return lambda f: f() if cond else None
    return pl.when(cond)


def _dot(a, b):
    return jnp.dot(a, b, preferred_element_type=F32)


def _dot_nt(a, b):
    return jax.lax.dot_general(a, b, (((1,), (1,)), ((), ())), preferred_element_type=F32)


def _kernel(x_hbm, mem0_ref, wq_hbm, wk_hbm, wv_hbm, wo_hbm, bqkv_hbm, bwo_hbm, gw_ref,
            out_hbm,
            x_vm, bqkv_vm, bwo_vm, perm_s, bwo_t, bqkv_p, bwo_p, stage, wqkv_s, wo_s,
            q_b, k_b, v_b, o_b, bmix, gate, out_vm, in_sem, x_sem, w_sem, out_sem,
            *, seg, dh):
    S, D = x_vm.shape
    M = mem0_ref.shape[0]
    L = M + seg
    n_seg = S // seg
    PW = 2 * dh
    n_pair = wo_hbm.shape[0] // PW
    n_blk = S // RB
    ppb = n_pair // n_blk
    nt = D // LANES
    bdh = D // B_HEADS

    cp_bqkv = [pltpu.make_async_copy(bqkv_hbm.at[:, j * D:(j + 1) * D], bqkv_vm.at[j], in_sem.at[j])
               for j in range(3)]
    cp_bwo = pltpu.make_async_copy(bwo_hbm, bwo_vm, in_sem.at[3])

    def x_copy(i):
        rows = pl.ds(_aligned(i * RB, RB), RB)
        return pltpu.make_async_copy(x_hbm.at[rows, :], x_vm.at[rows, :], x_sem.at[i])

    for c in (cp_bqkv[1], cp_bqkv[0], cp_bqkv[2], cp_bwo, x_copy(0)):
        c.start()

    def w_copies(g):
        rows = pl.ds(_aligned(g * (PW // 2), PW // 2), PW // 2)
        dsts = [stage.at[g, 0], stage.at[g, 1], stage.at[g, 2], wo_s.at[g]]
        return [pltpu.make_async_copy(src.bitcast(U32).at[rows, :], dsts[j], w_sem.at[g, j])
                for j, src in enumerate((wq_hbm, wk_hbm, wv_hbm, wo_hbm))]

    def start_batch(i):
        @_when(i + 1 < n_blk)
        def _():
            x_copy(i + 1).start()

        for t in range(ppb):
            for c in w_copies(i * ppb + t):
                c.start()

    def permuted_rows(ref):
        return jnp.concatenate(
            [ref[pl.ds(d, B_HEADS, stride=bdh), :] for d in range(bdh)], axis=0)

    for j in (1, 0, 2):
        if j == 1:
            cp_bqkv[1].wait()
            start_batch(0)
        elif j == 0:
            for c in (cp_bqkv[0], cp_bqkv[2], cp_bwo):
                c.wait()
        words = pltpu.bitcast(bqkv_vm[j], U32)
        for u, r in enumerate(range(0, D // 2, LANES)):
            n = min(LANES, D // 2 - r)
            blk = words[r:r + n, :]
            if n < LANES:
                blk = jnp.concatenate([blk] * (LANES // n), axis=0)
            perm_s[j, u] = blk.T
            bqkv_p[j, r:r + n, :] = permuted_rows(perm_s.at[j, u]).T[0:n, :]
    for t in range(nt):
        bwo_t[t] = bwo_vm[:, t * LANES:(t + 1) * LANES].astype(F32)
        bwo_p[:, t * LANES:(t + 1) * LANES] = pltpu.bitcast(
            permuted_rows(bwo_t.at[t]).astype(BF16), U32)

    a_scale = dh ** -0.5
    half = dh - LANES

    def out_copy(s):
        rows = pl.ds(_aligned(s * seg, seg), seg)
        return pltpu.make_async_copy(out_vm.at[rows, :], out_hbm.at[rows, :], out_sem.at[0])

    def block_diag(a):
        lo = _iota((L, LANES), 1) < half
        z = jnp.zeros((L, LANES), F32)
        mid = a[:, LANES:2 * LANES]
        top = jnp.concatenate([a[:, 0:LANES], jnp.where(lo, mid, 0.0), z], axis=1)
        bot = jnp.concatenate([z, jnp.where(lo, 0.0, mid), a[:, 2 * LANES:3 * LANES]], axis=1)
        return jnp.concatenate([top, bot], axis=0).astype(BF16)

    def a_rows(s, mem):
        row0 = _aligned(s * seg, seg)
        return jnp.concatenate([mem, x_vm[pl.ds(row0, seg), :].astype(F32)], axis=0)

    def a_project(h, g):
        return _dot(h, pltpu.bitcast(wqkv_s[g], BF16))

    def a_probs(qkv):
        row = _iota((L, 2 * L), 0)
        col = _iota((L, 2 * L), 1)
        first = col < L
        visible = (row < M) | (row >= jnp.where(first, col, col - L))
        sc = _dot_nt(qkv[:, 0:PW], block_diag(qkv[:, PW:2 * PW])) * a_scale
        sc = jnp.where(visible, sc, NEG)
        m0 = jnp.max(jnp.where(first, sc, -jnp.inf), axis=1, keepdims=True)
        m1 = jnp.max(jnp.where(first, -jnp.inf, sc), axis=1, keepdims=True)
        e = jnp.exp(sc - jnp.where(first, m0, m1))
        s0 = jnp.sum(jnp.where(first, e, 0.0), axis=1, keepdims=True)
        s1 = jnp.sum(jnp.where(first, 0.0, e), axis=1, keepdims=True)
        return e / jnp.where(first, s0, s1), block_diag(qkv[:, 2 * PW:3 * PW])

    def a_out(o, g):
        return _dot(o, pltpu.bitcast(wo_s[g], BF16))

    def a_finish(s, acc):
        rows = pl.ds(_aligned(s * seg, seg), seg)
        g = jnp.concatenate([gate[rows, :]] * nt, axis=1)
        out_vm[rows, :] = (g * acc[M:, :] + bmix[rows, :]).astype(BF16)
        out_copy(s).start()
        return acc[0:M, :]

    gw = gw_ref[...].astype(F32)
    b_scale = bdh ** -0.5

    def relayout(g):
        for j in range(3):
            wt = pltpu.bitcast(stage[g, j], BF16).T
            wqkv_s[g, :, j * PW:(j + 1) * PW] = pltpu.bitcast(wt, U32)

    def b_project(c, u):
        xb = x_vm[pl.ds(_aligned(c * RH, RH), RH), :]
        k = _dot(xb, pltpu.bitcast(bqkv_p[1], BF16))
        q_b[u] = _dot(xb, pltpu.bitcast(bqkv_p[0], BF16)) * b_scale
        v = _dot(xb, pltpu.bitcast(bqkv_p[2], BF16))
        for t in range(nt):
            k_b[u, t, HALO:HALO + RH, :] = k[:, t * LANES:(t + 1) * LANES]
            v_b[u, t, HALO:HALO + RH, :] = v[:, t * LANES:(t + 1) * LANES]

    def b_halo(u, first=False):
        for buf in (k_b, v_b):
            for t in range(nt):
                if first:
                    tail = jnp.broadcast_to(buf[u, t, HALO:HALO + 1, :], (HALO, LANES))
                else:
                    tail = buf[1 - u, t, RH:RH + HALO, :]
                buf[u, t, 0:HALO, :] = tail

    def b_attend(u, first=False):
        for r in range(0, RH, RS):
            base = HALO + r
            qs = [q_b[u, r:r + RS, t * LANES:(t + 1) * LANES] for t in range(nt)]
            logits = []
            for w in range(B_WIN):
                lo = base - w * B_DIL
                acc = qs[0] * k_b[u, 0, lo:lo + RS, :]
                for t in range(1, nt):
                    acc = acc + qs[t] * k_b[u, t, lo:lo + RS, :]
                acc = acc + pltpu.roll(acc, 2 * B_HEADS, 1)
                acc = acc + pltpu.roll(acc, B_HEADS, 1)
                if first and r < w * B_DIL:
                    acc = jnp.where(r + _iota((RS, LANES), 0) >= w * B_DIL, acc, NEG)
                logits.append(acc)
            mx = functools.reduce(jnp.maximum, logits)
            es = [jnp.exp(l - mx) for l in logits]
            inv = 1.0 / functools.reduce(jnp.add, es)
            ps = [e * inv for e in es]
            for t in range(nt):
                acc = ps[0] * v_b[u, t, base:base + RS, :]
                for w in range(1, B_WIN):
                    lo = base - w * B_DIL
                    acc = acc + ps[w] * v_b[u, t, lo:lo + RS, :]
                o_b[u, r:r + RS, t * LANES:(t + 1) * LANES] = acc.astype(BF16)

    def b_finish(c, u):
        rows = pl.ds(_aligned(c * RH, RH), RH)
        b = _dot(o_b[u], pltpu.bitcast(bwo_p[...], BF16))
        z = jnp.sum(x_vm[rows, :].astype(F32) * gw, axis=1, keepdims=True)
        g = 1.0 / (1.0 + jnp.exp(-z))
        gate[rows, :] = jnp.broadcast_to(g, (RH, LANES))
        bmix[rows, :] = (1.0 - g) * b

    def fetch(i):
        x_copy(i).wait()

        @_when(i + 1 < n_blk)
        def _():
            start_batch(i + 1)

    def arrived(i):
        gs = [i * ppb + t for t in range(ppb)]
        for g in gs:
            for c in w_copies(g):
                c.wait()
        return gs

    def b_block(i, acc):
        gs = arrived(i - 1)
        fetch(i)
        h = a_rows(0, mem0_ref[...].astype(F32))
        b_halo(1)
        b_attend(1)
        b_project(2 * i, 0)
        qkvs = []
        for g in gs:
            relayout(g)
            qkvs.append(a_project(h, g))
        b_finish(2 * i - 2, 0)
        pvs = [a_probs(qkv) for qkv in qkvs]
        b_halo(0)
        b_attend(0)
        b_project(2 * i + 1, 1)
        outs = [_dot(*pv) for pv in pvs]
        b_finish(2 * i - 1, 1)
        for g, o in zip(gs, outs):
            acc = acc + a_out(o, g)
        return acc

    fetch(0)
    b_project(0, 0)
    b_halo(0, first=True)
    b_attend(0, first=True)
    b_project(1, 1)
    acc0 = jax.lax.fori_loop(1, n_blk, b_block, jnp.zeros((L, D), F32))
    b_halo(1)
    b_attend(1)
    b_finish(2 * n_blk - 2, 0)
    b_finish(2 * n_blk - 1, 1)
    gs = arrived(n_blk - 1)
    h0 = a_rows(0, mem0_ref[...].astype(F32))
    qkvs = []
    for g in gs:
        relayout(g)
        qkvs.append(a_project(h0, g))
    pvs = [a_probs(qkv) for qkv in qkvs]
    for g, pv in zip(gs, pvs):
        acc0 = acc0 + a_out(_dot(*pv), g)

    def a_step(s, mem):
        h = a_rows(s, mem)
        qkvs, pvs, outs, acc = {}, {}, {}, None
        for t in range(n_pair + LAG2):
            if t == 0:
                qkvs[t] = functools.reduce(jnp.add, [
                    _dot(h[:, c * LANES:(c + 1) * LANES],
                         pltpu.bitcast(wqkv_s[t, c * LANES // 2:(c + 1) * LANES // 2, :], BF16))
                    for c in range(nt)])
            elif t < n_pair:
                qkvs[t] = a_project(h, t)
            if 0 <= t - LAG1 < n_pair:
                pvs[t - LAG1] = a_probs(qkvs.pop(t - LAG1))
            if 0 <= t - LAG2 < n_pair:
                outs[t - LAG2] = _dot(*pvs.pop(t - LAG2))
            g = t - LAG3
            if t >= n_pair:
                g = n_pair - LAG3 + (t - n_pair)
            if 0 <= g < n_pair - TAIL:
                y = a_out(outs.pop(g), g)
                acc = y if acc is None else acc + y
        left = sorted(outs)
        o = jnp.concatenate([outs[g] for g in left], axis=1)
        cols = []
        for c in range(nt):
            w = wo_s[left[0]:n_pair, :, c * LANES:(c + 1) * LANES].reshape(-1, LANES)
            cols.append(acc[:, c * LANES:(c + 1) * LANES] + _dot(o, pltpu.bitcast(w, BF16)))
        return a_finish(s, jnp.concatenate(cols, axis=1))

    def a_steps(i, mem):
        for u in range(UNROLL):
            mem = a_step(1 + i * UNROLL + u, mem)
        return mem

    assert (n_seg - 1) % UNROLL == 0
    jax.lax.fori_loop(0, (n_seg - 1) // UNROLL, a_steps, a_finish(0, acc0))
    pltpu.make_async_copy(out_vm, out_hbm, out_sem.at[0]).wait()


@functools.partial(jax.jit, static_argnames=("A_seg_len",))
def pallas_gated_mix__memory_aug_recurrent_mem_tr__sliding_local_dilated__prompt_kernel(
    A_x: jax.Array,
    A_mem0: jax.Array,
    A_Wq: jax.Array,
    A_Wk: jax.Array,
    A_Wv: jax.Array,
    A_Wo: jax.Array,
    A_seg_len: int,
    B_x: jax.Array,
    B_wqkv: jax.Array,
    B_wo: jax.Array,
    gate_w: jax.Array,
):
    del B_x
    _, S, D = A_x.shape
    _, H, dh = A_Wq.shape
    M = A_mem0.shape[1]
    PW = 2 * dh
    n_pair = H // 2

    def rows(w):
        return jnp.transpose(w, (1, 2, 0)).reshape(H * dh, D)

    hbm = pl.BlockSpec(memory_space=pl.ANY)
    vmem = pl.BlockSpec(memory_space=pltpu.VMEM)
    out = pl.pallas_call(
        functools.partial(_kernel, seg=int(A_seg_len), dh=dh),
        out_shape=jax.ShapeDtypeStruct((S, D), A_x.dtype),
        in_specs=[hbm, vmem, hbm, hbm, hbm, hbm, hbm, hbm, vmem],
        out_specs=hbm,
        scratch_shapes=[
            pltpu.VMEM((S, D), BF16),
            pltpu.VMEM((3, D, D), BF16),
            pltpu.VMEM((D, D), BF16),
            pltpu.VMEM((3, pl.cdiv(D // 2, LANES), D, LANES), U32),
            pltpu.VMEM((D // LANES, D, LANES), F32),
            pltpu.VMEM((3, D // 2, D), U32),
            pltpu.VMEM((D // 2, D), U32),
            pltpu.VMEM((n_pair, 3, PW // 2, D), U32),
            pltpu.VMEM((n_pair, D // 2, 3 * PW), U32),
            pltpu.VMEM((n_pair, PW // 2, D), U32),
            pltpu.VMEM((2, RH, D), F32),
            pltpu.VMEM((2, D // LANES, HALO + RH, LANES), F32),
            pltpu.VMEM((2, D // LANES, HALO + RH, LANES), F32),
            pltpu.VMEM((2, RH, D), BF16),
            pltpu.VMEM((S, D), F32),
            pltpu.VMEM((S, LANES), F32),
            pltpu.VMEM((S, D), BF16),
            pltpu.SemaphoreType.DMA((4,)),
            pltpu.SemaphoreType.DMA((S // RB,)),
            pltpu.SemaphoreType.DMA((n_pair, 4)),
            pltpu.SemaphoreType.DMA((1,)),
        ],
        compiler_params=pltpu.CompilerParams(vmem_limit_bytes=110 * 2**20),
    )(A_x.reshape(S, D), A_mem0.reshape(M, D), rows(A_Wq), rows(A_Wk), rows(A_Wv),
      A_Wo.reshape(H * dh, D), B_wqkv, B_wo, gate_w.reshape(1, D))
    return out.reshape(A_x.shape)
```

```python
import functools

import jax
import jax.numpy as jnp
import jax.experimental.pallas as pl
import jax.experimental.pallas.tpu as pltpu

F32 = jnp.float32
BF16 = jnp.bfloat16
U32 = jnp.uint32
NEG = -1000000000.0

B_HEADS = 32
B_WIN = 8
B_DIL = 2
HALO = 16
RB = 256
RH = 128
RS = 16
LANES = 128
LAG1, LAG2, LAG3 = 1, 4, 8
TAIL = 4
UNROLL = 3


def _iota(shape, dim):
    return jax.lax.broadcasted_iota(jnp.int32, shape, dim)


def _aligned(i, n):
    return i if isinstance(i, int) else pl.multiple_of(i, n)


def _when(cond):
    if isinstance(cond, bool):
        return lambda f: f() if cond else None
    return pl.when(cond)


def _dot(a, b):
    return jnp.dot(a, b, preferred_element_type=F32)


def _dot_nt(a, b):
    return jax.lax.dot_general(a, b, (((1,), (1,)), ((), ())), preferred_element_type=F32)


def _kernel(x_hbm, mem0_ref, wq_hbm, wk_hbm, wv_hbm, wo_hbm, bqkv_hbm, bwo_hbm, gw_ref,
            out_hbm,
            x_vm, bqkv_vm, bwo_vm, perm_s, bwo_t, bqkv_p, bwo_p, stage, wqkv_s, wo_s,
            q_b, k_b, v_b, o_b, bmix, gate, out_vm, in_sem, x_sem, w_sem, out_sem,
            *, seg, dh):
    S, D = x_vm.shape
    M = mem0_ref.shape[0]
    L = M + seg
    n_seg = S // seg
    PW = 2 * dh
    n_pair = wo_hbm.shape[0] // PW
    n_blk = S // RB
    ppb = n_pair // n_blk
    nt = D // LANES
    bdh = D // B_HEADS

    cp_bqkv = [pltpu.make_async_copy(bqkv_hbm.at[:, j * D:(j + 1) * D], bqkv_vm.at[j], in_sem.at[j])
               for j in range(3)]
    cp_bwo = pltpu.make_async_copy(bwo_hbm, bwo_vm, in_sem.at[3])

    def x_copy(i):
        rows = pl.ds(_aligned(i * RB, RB), RB)
        return pltpu.make_async_copy(x_hbm.at[rows, :], x_vm.at[rows, :], x_sem.at[i])

    for c in (cp_bqkv[1], x_copy(0), cp_bqkv[0], cp_bqkv[2], cp_bwo):
        c.start()

    def w_copies(g):
        rows = pl.ds(_aligned(g * (PW // 2), PW // 2), PW // 2)
        dsts = [stage.at[g, 0], stage.at[g, 1], stage.at[g, 2], wo_s.at[g]]
        return [pltpu.make_async_copy(src.bitcast(U32).at[rows, :], dsts[j], w_sem.at[g, j])
                for j, src in enumerate((wq_hbm, wk_hbm, wv_hbm, wo_hbm))]

    def start_batch(i):
        @_when(i + 1 < n_blk)
        def _():
            x_copy(i + 1).start()

        for t in range(ppb):
            for c in w_copies(i * ppb + t):
                c.start()

    def permuted_rows(ref):
        return jnp.concatenate(
            [ref[pl.ds(d, B_HEADS, stride=bdh), :] for d in range(bdh)], axis=0)

    def permute_qkv(j):
        words = pltpu.bitcast(bqkv_vm[j], U32)
        for u, r in enumerate(range(0, D // 2, LANES)):
            n = min(LANES, D // 2 - r)
            blk = words[r:r + n, :]
            if n < LANES:
                blk = jnp.concatenate([blk] * (LANES // n), axis=0)
            perm_s[j, u] = blk.T
            bqkv_p[j, r:r + n, :] = permuted_rows(perm_s.at[j, u]).T[0:n, :]

    def permute_wo():
        for t in range(nt):
            bwo_t[t] = bwo_vm[:, t * LANES:(t + 1) * LANES].astype(F32)
            bwo_p[:, t * LANES:(t + 1) * LANES] = pltpu.bitcast(
                permuted_rows(bwo_t.at[t]).astype(BF16), U32)

    a_scale = dh ** -0.5
    half = dh - LANES

    def out_copy(s):
        rows = pl.ds(_aligned(s * seg, seg), seg)
        return pltpu.make_async_copy(out_vm.at[rows, :], out_hbm.at[rows, :], out_sem.at[0])

    def block_diag(a):
        lo = _iota((L, LANES), 1) < half
        z = jnp.zeros((L, LANES), F32)
        mid = a[:, LANES:2 * LANES]
        top = jnp.concatenate([a[:, 0:LANES], jnp.where(lo, mid, 0.0), z], axis=1)
        bot = jnp.concatenate([z, jnp.where(lo, 0.0, mid), a[:, 2 * LANES:3 * LANES]], axis=1)
        return jnp.concatenate([top, bot], axis=0).astype(BF16)

    def a_rows(s, mem):
        row0 = _aligned(s * seg, seg)
        return jnp.concatenate([mem, x_vm[pl.ds(row0, seg), :].astype(F32)], axis=0)

    def a_project(h, g):
        return _dot(h, pltpu.bitcast(wqkv_s[g], BF16))

    def a_probs(qkv):
        row = _iota((L, 2 * L), 0)
        col = _iota((L, 2 * L), 1)
        first = col < L
        visible = (row < M) | (row >= jnp.where(first, col, col - L))
        sc = _dot_nt(qkv[:, 0:PW], block_diag(qkv[:, PW:2 * PW])) * a_scale
        sc = jnp.where(visible, sc, NEG)
        m0 = jnp.max(jnp.where(first, sc, -jnp.inf), axis=1, keepdims=True)
        m1 = jnp.max(jnp.where(first, -jnp.inf, sc), axis=1, keepdims=True)
        e = jnp.exp(sc - jnp.where(first, m0, m1))
        s0 = jnp.sum(jnp.where(first, e, 0.0), axis=1, keepdims=True)
        s1 = jnp.sum(jnp.where(first, 0.0, e), axis=1, keepdims=True)
        return e / jnp.where(first, s0, s1), block_diag(qkv[:, 2 * PW:3 * PW])

    def a_out(o, g):
        return _dot(o, pltpu.bitcast(wo_s[g], BF16))

    def a_finish(s, acc):
        rows = pl.ds(_aligned(s * seg, seg), seg)
        g = jnp.concatenate([gate[rows, :]] * nt, axis=1)
        out_vm[rows, :] = (g * acc[M:, :] + bmix[rows, :]).astype(BF16)
        out_copy(s).start()
        return acc[0:M, :]

    gw = gw_ref[...].astype(F32).reshape(1, D)
    b_scale = bdh ** -0.5

    def relayout(g):
        for j in range(3):
            wt = pltpu.bitcast(stage[g, j], BF16).T
            wqkv_s[g, :, j * PW:(j + 1) * PW] = pltpu.bitcast(wt, U32)

    def b_project(c, u, parts=(1, 0, 2)):
        xb = x_vm[pl.ds(_aligned(c * RH, RH), RH), :]
        for j in parts:
            y = _dot(xb, pltpu.bitcast(bqkv_p[j], BF16))
            if j == 0:
                q_b[u] = y * b_scale
            else:
                for t in range(nt):
                    (k_b, v_b)[j - 1][u, t, HALO:HALO + RH, :] = y[:, t * LANES:(t + 1) * LANES]

    def b_halo(u, first=False):
        for buf in (k_b, v_b):
            for t in range(nt):
                if first:
                    tail = jnp.broadcast_to(buf[u, t, HALO:HALO + 1, :], (HALO, LANES))
                else:
                    tail = buf[1 - u, t, RH:RH + HALO, :]
                buf[u, t, 0:HALO, :] = tail

    def b_attend(u, first=False):
        for r in range(0, RH, RS):
            base = HALO + r
            qs = [q_b[u, r:r + RS, t * LANES:(t + 1) * LANES] for t in range(nt)]
            logits = []
            for w in range(B_WIN):
                lo = base - w * B_DIL
                acc = qs[0] * k_b[u, 0, lo:lo + RS, :]
                for t in range(1, nt):
                    acc = acc + qs[t] * k_b[u, t, lo:lo + RS, :]
                acc = acc + pltpu.roll(acc, 2 * B_HEADS, 1)
                acc = acc + pltpu.roll(acc, B_HEADS, 1)
                if first and r < w * B_DIL:
                    acc = jnp.where(r + _iota((RS, LANES), 0) >= w * B_DIL, acc, NEG)
                logits.append(acc)
            mx = functools.reduce(jnp.maximum, logits)
            es = [jnp.exp(l - mx) for l in logits]
            inv = 1.0 / functools.reduce(jnp.add, es)
            ps = [e * inv for e in es]
            for t in range(nt):
                acc = ps[0] * v_b[u, t, base:base + RS, :]
                for w in range(1, B_WIN):
                    lo = base - w * B_DIL
                    acc = acc + ps[w] * v_b[u, t, lo:lo + RS, :]
                o_b[u, r:r + RS, t * LANES:(t + 1) * LANES] = acc.astype(BF16)

    def b_finish(c, u):
        rows = pl.ds(_aligned(c * RH, RH), RH)
        b = _dot(o_b[u], pltpu.bitcast(bwo_p[...], BF16))
        z = jnp.sum(x_vm[rows, :].astype(F32) * gw, axis=1, keepdims=True)
        g = 1.0 / (1.0 + jnp.exp(-z))
        gate[rows, :] = jnp.broadcast_to(g, (RH, LANES))
        bmix[rows, :] = (1.0 - g) * b

    def fetch(i):
        x_copy(i).wait()

        @_when(i + 1 < n_blk)
        def _():
            start_batch(i + 1)

    def arrived(i):
        gs = [i * ppb + t for t in range(ppb)]
        for g in gs:
            for c in w_copies(g):
                c.wait()
        return gs

    def b_block(i, acc):
        gs = arrived(i - 1)
        fetch(i)
        h = a_rows(0, mem0_ref[...].astype(F32))
        b_halo(1)
        b_attend(1)
        b_project(2 * i, 0)
        qkvs = []
        for g in gs:
            relayout(g)
            qkvs.append(a_project(h, g))
        b_finish(2 * i - 2, 0)
        pvs = [a_probs(qkv) for qkv in qkvs]
        b_halo(0)
        b_attend(0)
        b_project(2 * i + 1, 1)
        outs = [_dot(*pv) for pv in pvs]
        b_finish(2 * i - 1, 1)
        for g, o in zip(gs, outs):
            acc = acc + a_out(o, g)
        return acc

    cp_bqkv[1].wait()
    permute_qkv(1)
    start_batch(0)
    x_copy(0).wait()
    cp_bqkv[0].wait()
    permute_qkv(0)
    b_project(0, 0, (1,))
    b_project(1, 1, (1,))
    cp_bqkv[2].wait()
    cp_bwo.wait()
    permute_qkv(2)
    b_project(0, 0, (0,))
    b_project(1, 1, (0,))
    start_batch(1)
    permute_wo()
    b_project(0, 0, (2,))
    b_halo(0, first=True)
    b_attend(0, first=True)
    b_project(1, 1, (2,))
    acc0 = jax.lax.fori_loop(1, n_blk, b_block, jnp.zeros((L, D), F32))
    b_halo(1)
    b_attend(1)
    b_finish(2 * n_blk - 2, 0)
    b_finish(2 * n_blk - 1, 1)
    gs = arrived(n_blk - 1)
    h0 = a_rows(0, mem0_ref[...].astype(F32))
    qkvs = []
    for g in gs:
        relayout(g)
        qkvs.append(a_project(h0, g))
    pvs = [a_probs(qkv) for qkv in qkvs]
    for g, pv in zip(gs, pvs):
        acc0 = acc0 + a_out(_dot(*pv), g)

    def a_step(s, mem):
        h = a_rows(s, mem)
        qkvs, pvs, outs, acc = {}, {}, {}, None
        for t in range(n_pair + LAG2):
            if t == 0:
                qkvs[t] = functools.reduce(jnp.add, [
                    _dot(h[:, c * LANES:(c + 1) * LANES],
                         pltpu.bitcast(wqkv_s[t, c * LANES // 2:(c + 1) * LANES // 2, :], BF16))
                    for c in range(nt)])
            elif t < n_pair:
                qkvs[t] = a_project(h, t)
            if 0 <= t - LAG1 < n_pair:
                pvs[t - LAG1] = a_probs(qkvs.pop(t - LAG1))
            if 0 <= t - LAG2 < n_pair:
                outs[t - LAG2] = _dot(*pvs.pop(t - LAG2))
            g = t - LAG3
            if t >= n_pair:
                g = n_pair - LAG3 + (t - n_pair)
            if 0 <= g < n_pair - TAIL:
                y = a_out(outs.pop(g), g)
                acc = y if acc is None else acc + y
        left = sorted(outs)
        o = jnp.concatenate([outs[g] for g in left], axis=1)
        cols = []
        for c in range(nt):
            w = wo_s[left[0]:n_pair, :, c * LANES:(c + 1) * LANES].reshape(-1, LANES)
            cols.append(acc[:, c * LANES:(c + 1) * LANES] + _dot(o, pltpu.bitcast(w, BF16)))
        return a_finish(s, jnp.concatenate(cols, axis=1))

    def a_steps(i, mem):
        for u in range(UNROLL):
            mem = a_step(1 + i * UNROLL + u, mem)
        return mem

    assert (n_seg - 1) % UNROLL == 0
    jax.lax.fori_loop(0, (n_seg - 1) // UNROLL, a_steps, a_finish(0, acc0))
    pltpu.make_async_copy(out_vm, out_hbm, out_sem.at[0]).wait()


@functools.partial(jax.jit, static_argnames=("A_seg_len",))
def pallas_gated_mix__memory_aug_recurrent_mem_tr__sliding_local_dilated__prompt_kernel(
    A_x: jax.Array,
    A_mem0: jax.Array,
    A_Wq: jax.Array,
    A_Wk: jax.Array,
    A_Wv: jax.Array,
    A_Wo: jax.Array,
    A_seg_len: int,
    B_x: jax.Array,
    B_wqkv: jax.Array,
    B_wo: jax.Array,
    gate_w: jax.Array,
):
    del B_x
    _, S, D = A_x.shape
    _, H, dh = A_Wq.shape
    M = A_mem0.shape[1]
    PW = 2 * dh
    n_pair = H // 2

    def rows(w):
        return jnp.transpose(w, (1, 2, 0)).reshape(H * dh, D)

    hbm = pl.BlockSpec(memory_space=pl.ANY)
    vmem = pl.BlockSpec(memory_space=pltpu.VMEM)
    out = pl.pallas_call(
        functools.partial(_kernel, seg=int(A_seg_len), dh=dh),
        out_shape=jax.ShapeDtypeStruct((S, D), A_x.dtype),
        in_specs=[hbm, vmem, hbm, hbm, hbm, hbm, hbm, hbm, vmem],
        out_specs=hbm,
        scratch_shapes=[
            pltpu.VMEM((S, D), BF16),
            pltpu.VMEM((3, D, D), BF16),
            pltpu.VMEM((D, D), BF16),
            pltpu.VMEM((3, pl.cdiv(D // 2, LANES), D, LANES), U32),
            pltpu.VMEM((D // LANES, D, LANES), F32),
            pltpu.VMEM((3, D // 2, D), U32),
            pltpu.VMEM((D // 2, D), U32),
            pltpu.VMEM((n_pair, 3, PW // 2, D), U32),
            pltpu.VMEM((n_pair, D // 2, 3 * PW), U32),
            pltpu.VMEM((n_pair, PW // 2, D), U32),
            pltpu.VMEM((2, RH, D), F32),
            pltpu.VMEM((2, D // LANES, HALO + RH, LANES), F32),
            pltpu.VMEM((2, D // LANES, HALO + RH, LANES), F32),
            pltpu.VMEM((2, RH, D), BF16),
            pltpu.VMEM((S, D), F32),
            pltpu.VMEM((S, LANES), F32),
            pltpu.VMEM((S, D), BF16),
            pltpu.SemaphoreType.DMA((4,)),
            pltpu.SemaphoreType.DMA((S // RB,)),
            pltpu.SemaphoreType.DMA((n_pair, 4)),
            pltpu.SemaphoreType.DMA((1,)),
        ],
        compiler_params=pltpu.CompilerParams(vmem_limit_bytes=110 * 2**20),
    )(A_x.reshape(S, D), A_mem0.reshape(M, D), rows(A_Wq), rows(A_Wk), rows(A_Wv),
      A_Wo.reshape(H * dh, D), B_wqkv, B_wo, gate_w)
    return out.reshape(A_x.shape)
```

```python
import functools

import jax
import jax.numpy as jnp
import jax.experimental.pallas as pl
import jax.experimental.pallas.tpu as pltpu

F32 = jnp.float32
BF16 = jnp.bfloat16
U32 = jnp.uint32
NEG = -1000000000.0

B_HEADS = 32
B_WIN = 8
B_DIL = 2
HALO = 16
RB = 256
RH = 128
RS = 16
LANES = 128
LAG1, LAG2, LAG3 = 1, 4, 8
TAIL = 4
UNROLL = 3


def _iota(shape, dim):
    return jax.lax.broadcasted_iota(jnp.int32, shape, dim)


def _aligned(i, n):
    return i if isinstance(i, int) else pl.multiple_of(i, n)


def _when(cond):
    if isinstance(cond, bool):
        return lambda f: f() if cond else None
    return pl.when(cond)


def _dot(a, b):
    return jnp.dot(a, b, preferred_element_type=F32)


def _dot_nt(a, b):
    return jax.lax.dot_general(a, b, (((1,), (1,)), ((), ())), preferred_element_type=F32)


def _kernel(x_hbm, mem0_ref, wq_hbm, wk_hbm, wv_hbm, wo_hbm, bqkv_hbm, bwo_hbm, gw_ref,
            out_hbm,
            x_vm, bqkv_vm, bwo_vm, perm_s, bwo_t, bqkv_p, bwo_p, stage, wqkv_s, wo_s,
            q_b, k_b, v_b, o_b, b_out, out_vm, in_sem, x_sem, w_sem, out_sem,
            *, seg, dh):
    S, D = x_vm.shape
    M = mem0_ref.shape[0]
    L = M + seg
    n_seg = S // seg
    PW = 2 * dh
    n_pair = wo_hbm.shape[0] // PW
    n_blk = S // RB
    ppb = n_pair // n_blk
    nt = D // LANES
    bdh = D // B_HEADS

    cp_bqkv = [pltpu.make_async_copy(bqkv_hbm.at[:, j * D:(j + 1) * D], bqkv_vm.at[j], in_sem.at[j])
               for j in range(3)]
    cp_bwo = pltpu.make_async_copy(bwo_hbm, bwo_vm, in_sem.at[3])

    def x_copy(i):
        rows = pl.ds(_aligned(i * RB, RB), RB)
        return pltpu.make_async_copy(x_hbm.at[rows, :], x_vm.at[rows, :], x_sem.at[i])

    for c in (cp_bqkv[1], x_copy(0), cp_bqkv[0], cp_bqkv[2], cp_bwo):
        c.start()

    def w_copies(g):
        rows = pl.ds(_aligned(g * (PW // 2), PW // 2), PW // 2)
        dsts = [stage.at[g, 0], stage.at[g, 1], stage.at[g, 2], wo_s.at[g]]
        return [pltpu.make_async_copy(src.bitcast(U32).at[rows, :], dsts[j], w_sem.at[g, j])
                for j, src in enumerate((wq_hbm, wk_hbm, wv_hbm, wo_hbm))]

    def start_batch(i):
        @_when(i + 1 < n_blk)
        def _():
            x_copy(i + 1).start()

        for t in range(ppb):
            for c in w_copies(i * ppb + t):
                c.start()

    def permuted_rows(ref):
        return jnp.concatenate(
            [ref[pl.ds(d, B_HEADS, stride=bdh), :] for d in range(bdh)], axis=0)

    def permute_qkv(j):
        words = pltpu.bitcast(bqkv_vm[j], U32)
        for u, r in enumerate(range(0, D // 2, LANES)):
            n = min(LANES, D // 2 - r)
            blk = words[r:r + n, :]
            if n < LANES:
                blk = jnp.concatenate([blk] * (LANES // n), axis=0)
            perm_s[j, u, 0:D, :] = blk.T
            bqkv_p[j, r:r + n, :] = permuted_rows(perm_s.at[j, u]).T[0:n, :]

    def permute_wo():
        for t in range(nt):
            bwo_t[t, 0:D, :] = bwo_vm[:, t * LANES:(t + 1) * LANES].astype(F32)
            bwo_p[:, t * LANES:(t + 1) * LANES] = pltpu.bitcast(
                permuted_rows(bwo_t.at[t]).astype(BF16), U32)

    a_scale = dh ** -0.5
    half = dh - LANES

    def out_copy(s):
        rows = pl.ds(_aligned(s * seg, seg), seg)
        return pltpu.make_async_copy(out_vm.at[rows, :], out_hbm.at[rows, :], out_sem.at[0])

    def block_diag(a):
        lo = _iota((L, LANES), 1) < half
        z = jnp.zeros((L, LANES), F32)
        mid = a[:, LANES:2 * LANES]
        top = jnp.concatenate([a[:, 0:LANES], jnp.where(lo, mid, 0.0), z], axis=1)
        bot = jnp.concatenate([z, jnp.where(lo, 0.0, mid), a[:, 2 * LANES:3 * LANES]], axis=1)
        return jnp.concatenate([top, bot], axis=0).astype(BF16)

    def a_rows(s, mem):
        row0 = _aligned(s * seg, seg)
        return jnp.concatenate([mem, x_vm[pl.ds(row0, seg), :].astype(F32)], axis=0)

    def a_project(h, g):
        return _dot(h, pltpu.bitcast(wqkv_s[g], BF16))

    def a_probs(qkv):
        row = _iota((L, 2 * L), 0)
        col = _iota((L, 2 * L), 1)
        first = col < L
        visible = (row < M) | (row >= jnp.where(first, col, col - L))
        sc = _dot_nt(qkv[:, 0:PW], block_diag(qkv[:, PW:2 * PW])) * a_scale
        sc = jnp.where(visible, sc, NEG)
        m0 = jnp.max(jnp.where(first, sc, -jnp.inf), axis=1, keepdims=True)
        m1 = jnp.max(jnp.where(first, -jnp.inf, sc), axis=1, keepdims=True)
        e = jnp.exp(sc - jnp.where(first, m0, m1))
        s0 = jnp.sum(jnp.where(first, e, 0.0), axis=1, keepdims=True)
        s1 = jnp.sum(jnp.where(first, 0.0, e), axis=1, keepdims=True)
        return e / jnp.where(first, s0, s1), block_diag(qkv[:, 2 * PW:3 * PW])

    def a_out(o, g):
        return _dot(o, pltpu.bitcast(wo_s[g], BF16))

    def a_finish(s, h, acc):
        rows = pl.ds(_aligned(s * seg, seg), seg)
        gw = gw_ref[...].astype(F32).reshape(1, D)
        z = jnp.sum(h[M:, :] * gw, axis=1, keepdims=True)
        g = 1.0 / (1.0 + jnp.exp(-z))
        out_vm[rows, :] = (g * acc[M:, :] + (1.0 - g) * b_out[rows, :]).astype(BF16)
        out_copy(s).start()
        return acc[0:M, :]

    b_scale = bdh ** -0.5

    def relayout(g):
        for j in range(3):
            wt = pltpu.bitcast(stage[g, j], BF16).T
            wqkv_s[g, :, j * PW:(j + 1) * PW] = pltpu.bitcast(wt, U32)

    def b_project(c, u, parts=(1, 0, 2)):
        xb = x_vm[pl.ds(_aligned(c * RH, RH), RH), :]
        for j in parts:
            y = _dot(xb, pltpu.bitcast(bqkv_p[j], BF16))
            if j == 0:
                q_b[u] = y * b_scale
            else:
                for t in range(nt):
                    (k_b, v_b)[j - 1][u, t, HALO:HALO + RH, :] = y[:, t * LANES:(t + 1) * LANES]

    def b_halo(u, first=False):
        for buf in (k_b, v_b):
            for t in range(nt):
                if first:
                    tail = jnp.broadcast_to(buf[u, t, HALO:HALO + 1, :], (HALO, LANES))
                else:
                    tail = buf[1 - u, t, RH:RH + HALO, :]
                buf[u, t, 0:HALO, :] = tail

    def b_attend(u, first=False):
        for r in range(0, RH, RS):
            base = HALO + r
            qs = [q_b[u, r:r + RS, t * LANES:(t + 1) * LANES] for t in range(nt)]
            logits = []
            for w in range(B_WIN):
                lo = base - w * B_DIL
                acc = qs[0] * k_b[u, 0, lo:lo + RS, :]
                for t in range(1, nt):
                    acc = acc + qs[t] * k_b[u, t, lo:lo + RS, :]
                acc = acc + pltpu.roll(acc, 2 * B_HEADS, 1)
                acc = acc + pltpu.roll(acc, B_HEADS, 1)
                if first and r < w * B_DIL:
                    acc = jnp.where(r + _iota((RS, LANES), 0) >= w * B_DIL, acc, NEG)
                logits.append(acc)
            mx = functools.reduce(jnp.maximum, logits)
            es = [jnp.exp(l - mx) for l in logits]
            inv = 1.0 / functools.reduce(jnp.add, es)
            ps = [e * inv for e in es]
            for t in range(nt):
                acc = ps[0] * v_b[u, t, base:base + RS, :]
                for w in range(1, B_WIN):
                    lo = base - w * B_DIL
                    acc = acc + ps[w] * v_b[u, t, lo:lo + RS, :]
                o_b[u, r:r + RS, t * LANES:(t + 1) * LANES] = acc.astype(BF16)

    def b_finish(c, u):
        rows = pl.ds(_aligned(c * RH, RH), RH)
        b_out[rows, :] = _dot(o_b[u], pltpu.bitcast(bwo_p[...], BF16))

    def fetch(i):
        x_copy(i).wait()

        @_when(i + 1 < n_blk)
        def _():
            start_batch(i + 1)

    def arrived(i):
        gs = [i * ppb + t for t in range(ppb)]
        for g in gs:
            for c in w_copies(g):
                c.wait()
        return gs

    def b_block(i, acc):
        gs = arrived(i - 1)
        fetch(i)
        h = a_rows(0, mem0_ref[...].astype(F32))
        b_halo(1)
        b_attend(1)
        b_project(2 * i, 0)
        qkvs = []
        for g in gs:
            relayout(g)
            qkvs.append(a_project(h, g))
        b_finish(2 * i - 2, 0)
        pvs = [a_probs(qkv) for qkv in qkvs]
        b_halo(0)
        b_attend(0)
        b_project(2 * i + 1, 1)
        outs = [_dot(*pv) for pv in pvs]
        b_finish(2 * i - 1, 1)
        for g, o in zip(gs, outs):
            acc = acc + a_out(o, g)
        return acc

    cp_bqkv[1].wait()
    permute_qkv(1)
    start_batch(0)
    x_copy(0).wait()
    cp_bqkv[0].wait()
    permute_qkv(0)
    b_project(0, 0, (1,))
    b_project(1, 1, (1,))
    cp_bqkv[2].wait()
    cp_bwo.wait()
    permute_qkv(2)
    b_project(0, 0, (0,))
    b_project(1, 1, (0,))
    start_batch(1)
    permute_wo()
    b_project(0, 0, (2,))
    b_halo(0, first=True)
    b_attend(0, first=True)
    b_project(1, 1, (2,))
    acc0 = jax.lax.fori_loop(1, n_blk, b_block, jnp.zeros((L, D), F32))
    b_halo(1)
    b_attend(1)
    b_finish(2 * n_blk - 2, 0)
    b_finish(2 * n_blk - 1, 1)
    gs = arrived(n_blk - 1)
    h0 = a_rows(0, mem0_ref[...].astype(F32))
    qkvs = []
    for g in gs:
        relayout(g)
        qkvs.append(a_project(h0, g))
    pvs = [a_probs(qkv) for qkv in qkvs]
    for g, pv in zip(gs, pvs):
        acc0 = acc0 + a_out(_dot(*pv), g)

    def a_step(s, mem):
        h = a_rows(s, mem)
        qkvs, pvs, outs, acc = {}, {}, {}, None
        for t in range(n_pair + LAG2):
            if t == 0:
                qkvs[t] = functools.reduce(jnp.add, [
                    _dot(h[:, c * LANES:(c + 1) * LANES],
                         pltpu.bitcast(wqkv_s[t, c * LANES // 2:(c + 1) * LANES // 2, :], BF16))
                    for c in range(nt)])
            elif t < n_pair:
                qkvs[t] = a_project(h, t)
            if 0 <= t - LAG1 < n_pair:
                pvs[t - LAG1] = a_probs(qkvs.pop(t - LAG1))
            if 0 <= t - LAG2 < n_pair:
                outs[t - LAG2] = _dot(*pvs.pop(t - LAG2))
            g = t - LAG3
            if t >= n_pair:
                g = n_pair - LAG3 + (t - n_pair)
            if 0 <= g < n_pair - TAIL:
                y = a_out(outs.pop(g), g)
                acc = y if acc is None else acc + y
        left = sorted(outs)
        o = jnp.concatenate([outs[g] for g in left], axis=1)
        cols = []
        for c in range(nt):
            w = wo_s[left[0]:n_pair, :, c * LANES:(c + 1) * LANES].reshape(-1, LANES)
            cols.append(acc[:, c * LANES:(c + 1) * LANES] + _dot(o, pltpu.bitcast(w, BF16)))
        return a_finish(s, h, jnp.concatenate(cols, axis=1))

    def a_steps(i, mem):
        for u in range(UNROLL):
            mem = a_step(1 + i * UNROLL + u, mem)
        return mem

    assert (n_seg - 1) % UNROLL == 0
    jax.lax.fori_loop(0, (n_seg - 1) // UNROLL, a_steps, a_finish(0, h0, acc0))
    pltpu.make_async_copy(out_vm, out_hbm, out_sem.at[0]).wait()


@functools.partial(jax.jit, static_argnames=("A_seg_len",))
def pallas_gated_mix__memory_aug_recurrent_mem_tr__sliding_local_dilated__prompt_kernel(
    A_x: jax.Array,
    A_mem0: jax.Array,
    A_Wq: jax.Array,
    A_Wk: jax.Array,
    A_Wv: jax.Array,
    A_Wo: jax.Array,
    A_seg_len: int,
    B_x: jax.Array,
    B_wqkv: jax.Array,
    B_wo: jax.Array,
    gate_w: jax.Array,
):
    del B_x
    _, S, D = A_x.shape
    _, H, dh = A_Wq.shape
    M = A_mem0.shape[1]
    PW = 2 * dh
    n_pair = H // 2

    def rows(w):
        return jnp.transpose(w, (1, 2, 0)).reshape(H * dh, D)

    hbm = pl.BlockSpec(memory_space=pl.ANY)
    vmem = pl.BlockSpec(memory_space=pltpu.VMEM)
    out = pl.pallas_call(
        functools.partial(_kernel, seg=int(A_seg_len), dh=dh),
        out_shape=jax.ShapeDtypeStruct((S, D), A_x.dtype),
        in_specs=[hbm, vmem, hbm, hbm, hbm, hbm, hbm, hbm, vmem],
        out_specs=hbm,
        scratch_shapes=[
            pltpu.VMEM((S, D), BF16),
            pltpu.VMEM((3, D, D), BF16),
            pltpu.VMEM((D, D), BF16),
            pltpu.VMEM((3, pl.cdiv(D // 2, LANES), D + 32, LANES), U32),
            pltpu.VMEM((D // LANES, D + 32, LANES), F32),
            pltpu.VMEM((3, D // 2, D), U32),
            pltpu.VMEM((D // 2, D), U32),
            pltpu.VMEM((n_pair, 3, PW // 2, D), U32),
            pltpu.VMEM((n_pair, D // 2, 3 * PW), U32),
            pltpu.VMEM((n_pair, PW // 2, D), U32),
            pltpu.VMEM((2, RH, D), F32),
            pltpu.VMEM((2, D // LANES, HALO + RH, LANES), F32),
            pltpu.VMEM((2, D // LANES, HALO + RH, LANES), F32),
            pltpu.VMEM((2, RH, D), BF16),
            pltpu.VMEM((S, D), F32),
            pltpu.VMEM((S, D), BF16),
            pltpu.SemaphoreType.DMA((4,)),
            pltpu.SemaphoreType.DMA((S // RB,)),
            pltpu.SemaphoreType.DMA((n_pair, 4)),
            pltpu.SemaphoreType.DMA((1,)),
        ],
        compiler_params=pltpu.CompilerParams(vmem_limit_bytes=110 * 2**20),
    )(A_x.reshape(S, D), A_mem0.reshape(M, D), rows(A_Wq), rows(A_Wk), rows(A_Wv),
      A_Wo.reshape(H * dh, D), B_wqkv, B_wo, gate_w)
    return out.reshape(A_x.shape)
```

```python
import functools

import jax
import jax.numpy as jnp
import jax.experimental.pallas as pl
import jax.experimental.pallas.tpu as pltpu

F32 = jnp.float32
BF16 = jnp.bfloat16
U32 = jnp.uint32
NEG = -1000000000.0

B_HEADS = 32
B_WIN = 8
B_DIL = 2
HALO = 16
RB = 256
RH = 128
RS = 16
LANES = 128
LAG1, LAG2, LAG3 = 1, 4, 8
TAIL = 4
UNROLL = 3


def _iota(shape, dim):
    return jax.lax.broadcasted_iota(jnp.int32, shape, dim)


def _aligned(i, n):
    return i if isinstance(i, int) else pl.multiple_of(i, n)


def _when(cond):
    if isinstance(cond, bool):
        return lambda f: f() if cond else None
    return pl.when(cond)


def _dot(a, b):
    return jnp.dot(a, b, preferred_element_type=F32)


def _dot_nt(a, b):
    return jax.lax.dot_general(a, b, (((1,), (1,)), ((), ())), preferred_element_type=F32)


def _kernel(x_hbm, mem0_ref, wq_hbm, wk_hbm, wv_hbm, wo_hbm, bqkv_hbm, bwo_hbm, gw_ref,
            out_hbm,
            x_vm, bqkv_vm, bwo_vm, perm_s, bwo_t, bqkv_p, bwo_p, stage, wqkv_s, wo_s,
            q_b, k_b, v_b, o_b, b_out, out_vm, in_sem, x_sem, w_sem, out_sem,
            *, seg, dh):
    S, D = x_vm.shape
    M = mem0_ref.shape[0]
    L = M + seg
    n_seg = S // seg
    PW = 2 * dh
    n_pair = wo_hbm.shape[0] // PW
    n_blk = S // RB
    ppb = n_pair // n_blk
    nt = D // LANES
    bdh = D // B_HEADS

    cp_bqkv = [pltpu.make_async_copy(bqkv_hbm.at[:, j * D:(j + 1) * D], bqkv_vm.at[j], in_sem.at[j])
               for j in range(3)]
    cp_bwo = pltpu.make_async_copy(bwo_hbm, bwo_vm, in_sem.at[3])

    def x_copy(i):
        rows = pl.ds(_aligned(i * RB, RB), RB)
        return pltpu.make_async_copy(x_hbm.at[rows, :], x_vm.at[rows, :], x_sem.at[i])

    for c in (cp_bqkv[1], x_copy(0), cp_bqkv[0], cp_bqkv[2], cp_bwo):
        c.start()

    def w_copies(g):
        rows = pl.ds(_aligned(g * (PW // 2), PW // 2), PW // 2)
        dsts = [stage.at[g, 0], stage.at[g, 1], stage.at[g, 2], wo_s.at[g]]
        return [pltpu.make_async_copy(src.bitcast(U32).at[rows, :], dsts[j], w_sem.at[g, j])
                for j, src in enumerate((wq_hbm, wk_hbm, wv_hbm, wo_hbm))]

    def start_batch(i):
        @_when(i + 1 < n_blk)
        def _():
            x_copy(i + 1).start()

        for t in range(ppb):
            for c in w_copies(i * ppb + t):
                c.start()

    def permuted_rows(ref):
        return jnp.concatenate(
            [ref[pl.ds(d, B_HEADS, stride=bdh), :] for d in range(bdh)], axis=0)

    def permute_qkv(j):
        words = pltpu.bitcast(bqkv_vm[j], U32)
        for u, r in enumerate(range(0, D // 2, LANES)):
            n = min(LANES, D // 2 - r)
            blk = words[r:r + n, :]
            if n < LANES:
                blk = jnp.concatenate([blk] * (LANES // n), axis=0)
            perm_s[j, u, 0:D, :] = blk.T
            bqkv_p[j, r:r + n, :] = permuted_rows(perm_s.at[j, u]).T[0:n, :]

    def permute_wo():
        for t in range(nt):
            bwo_t[t, 0:D, :] = bwo_vm[:, t * LANES:(t + 1) * LANES].astype(F32)
            bwo_p[:, t * LANES:(t + 1) * LANES] = pltpu.bitcast(
                permuted_rows(bwo_t.at[t]).astype(BF16), U32)

    a_scale = dh ** -0.5
    half = dh - LANES

    def out_copy(s):
        rows = pl.ds(_aligned(s * seg, seg), seg)
        return pltpu.make_async_copy(out_vm.at[rows, :], out_hbm.at[rows, :], out_sem.at[0])

    def block_diag(a):
        lo = _iota((L, LANES), 1) < half
        z = jnp.zeros((L, LANES), F32)
        mid = a[:, LANES:2 * LANES]
        top = jnp.concatenate([a[:, 0:LANES], jnp.where(lo, mid, 0.0), z], axis=1)
        bot = jnp.concatenate([z, jnp.where(lo, 0.0, mid), a[:, 2 * LANES:3 * LANES]], axis=1)
        return jnp.concatenate([top, bot], axis=0).astype(BF16)

    def a_rows(s, mem):
        row0 = _aligned(s * seg, seg)
        return jnp.concatenate([mem, x_vm[pl.ds(row0, seg), :].astype(F32)], axis=0)

    def a_project(h, g):
        return _dot(h, pltpu.bitcast(wqkv_s[g], BF16))

    def a_probs(qkv):
        row = _iota((L, 2 * L), 0)
        col = _iota((L, 2 * L), 1)
        first = col < L
        visible = (row < M) | (row >= jnp.where(first, col, col - L))
        sc = _dot_nt(qkv[:, 0:PW], block_diag(qkv[:, PW:2 * PW])) * a_scale
        sc = jnp.where(visible, sc, NEG)
        m0 = jnp.max(jnp.where(first, sc, -jnp.inf), axis=1, keepdims=True)
        m1 = jnp.max(jnp.where(first, -jnp.inf, sc), axis=1, keepdims=True)
        e = jnp.exp(sc - jnp.where(first, m0, m1))
        s0 = jnp.sum(jnp.where(first, e, 0.0), axis=1, keepdims=True)
        s1 = jnp.sum(jnp.where(first, 0.0, e), axis=1, keepdims=True)
        return e / jnp.where(first, s0, s1), block_diag(qkv[:, 2 * PW:3 * PW])

    def a_out(o, g):
        return _dot(o, pltpu.bitcast(wo_s[g], BF16))

    def a_finish(s, h, acc):
        rows = pl.ds(_aligned(s * seg, seg), seg)
        gw = gw_ref[...].astype(F32).reshape(1, D)
        z = jnp.sum(h[M:, :] * gw, axis=1, keepdims=True)
        g = 1.0 / (1.0 + jnp.exp(-z))
        out_vm[rows, :] = (g * acc[M:, :] + (1.0 - g) * b_out[rows, :]).astype(BF16)
        out_copy(s).start()
        return acc[0:M, :]

    b_scale = bdh ** -0.5

    def relayout(g):
        for j in range(3):
            wt = pltpu.bitcast(stage[g, j], BF16).T
            wqkv_s[g, :, j * PW:(j + 1) * PW] = pltpu.bitcast(wt, U32)

    def b_project(c, u, parts=(1, 0, 2)):
        xb = x_vm[pl.ds(_aligned(c * RH, RH), RH), :]
        for j in parts:
            y = _dot(xb, pltpu.bitcast(bqkv_p[j], BF16))
            if j == 0:
                q_b[u][...] = y * b_scale
            else:
                for t in range(nt):
                    (k_b, v_b)[j - 1][u][t, HALO:HALO + RH, :] = y[:, t * LANES:(t + 1) * LANES]

    def b_halo(u, first=False):
        for buf in (k_b, v_b):
            for t in range(nt):
                if first:
                    tail = jnp.broadcast_to(buf[u][t, HALO:HALO + 1, :], (HALO, LANES))
                else:
                    tail = buf[1 - u][t, RH:RH + HALO, :]
                buf[u][t, 0:HALO, :] = tail

    def b_attend(u, first=False):
        for r in range(0, RH, RS):
            base = HALO + r
            qs = [q_b[u][r:r + RS, t * LANES:(t + 1) * LANES] for t in range(nt)]
            logits = []
            for w in range(B_WIN):
                lo = base - w * B_DIL
                acc = qs[0] * k_b[u][0, lo:lo + RS, :]
                for t in range(1, nt):
                    acc = acc + qs[t] * k_b[u][t, lo:lo + RS, :]
                acc = acc + pltpu.roll(acc, 2 * B_HEADS, 1)
                acc = acc + pltpu.roll(acc, B_HEADS, 1)
                if first and r < w * B_DIL:
                    acc = jnp.where(r + _iota((RS, LANES), 0) >= w * B_DIL, acc, NEG)
                logits.append(acc)
            mx = functools.reduce(jnp.maximum, logits)
            es = [jnp.exp(l - mx) for l in logits]
            inv = 1.0 / functools.reduce(jnp.add, es)
            ps = [e * inv for e in es]
            for t in range(nt):
                acc = ps[0] * v_b[u][t, base:base + RS, :]
                for w in range(1, B_WIN):
                    lo = base - w * B_DIL
                    acc = acc + ps[w] * v_b[u][t, lo:lo + RS, :]
                o_b[u][r:r + RS, t * LANES:(t + 1) * LANES] = acc.astype(BF16)

    def b_finish(c, u):
        rows = pl.ds(_aligned(c * RH, RH), RH)
        b_out[rows, :] = _dot(o_b[u][...], pltpu.bitcast(bwo_p[...], BF16))

    def fetch(i):
        x_copy(i).wait()

        @_when(i + 1 < n_blk)
        def _():
            start_batch(i + 1)

    def arrived(i):
        gs = [i * ppb + t for t in range(ppb)]
        for g in gs:
            for c in w_copies(g):
                c.wait()
        return gs

    def b_block(i, acc):
        gs = arrived(i - 1)
        fetch(i)
        h = a_rows(0, mem0_ref[...].astype(F32))
        b_halo(1)
        b_attend(1)
        b_project(2 * i, 0)
        qkvs = []
        for g in gs:
            relayout(g)
            qkvs.append(a_project(h, g))
        b_finish(2 * i - 2, 0)
        pvs = [a_probs(qkv) for qkv in qkvs]
        b_halo(0)
        b_attend(0)
        b_project(2 * i + 1, 1)
        outs = [_dot(*pv) for pv in pvs]
        b_finish(2 * i - 1, 1)
        for g, o in zip(gs, outs):
            acc = acc + a_out(o, g)
        return acc

    cp_bqkv[1].wait()
    permute_qkv(1)
    start_batch(0)
    x_copy(0).wait()
    cp_bqkv[0].wait()
    permute_qkv(0)
    b_project(0, 0, (1,))
    b_project(1, 1, (1,))
    cp_bqkv[2].wait()
    cp_bwo.wait()
    permute_qkv(2)
    b_project(0, 0, (0,))
    b_project(1, 1, (0,))
    start_batch(1)
    permute_wo()
    b_project(0, 0, (2,))
    b_halo(0, first=True)
    b_attend(0, first=True)
    b_project(1, 1, (2,))
    acc0 = jax.lax.fori_loop(1, n_blk, b_block, jnp.zeros((L, D), F32))
    b_halo(1)
    b_attend(1)
    b_finish(2 * n_blk - 2, 0)
    b_finish(2 * n_blk - 1, 1)
    gs = arrived(n_blk - 1)
    h0 = a_rows(0, mem0_ref[...].astype(F32))
    qkvs = []
    for g in gs:
        relayout(g)
        qkvs.append(a_project(h0, g))
    pvs = [a_probs(qkv) for qkv in qkvs]
    for g, pv in zip(gs, pvs):
        acc0 = acc0 + a_out(_dot(*pv), g)

    def a_step(s, mem):
        h = a_rows(s, mem)
        qkvs, pvs, outs, acc = {}, {}, {}, None
        for t in range(n_pair + LAG2):
            if t == 0:
                qkvs[t] = functools.reduce(jnp.add, [
                    _dot(h[:, c * LANES:(c + 1) * LANES],
                         pltpu.bitcast(wqkv_s[t, c * LANES // 2:(c + 1) * LANES // 2, :], BF16))
                    for c in range(nt)])
            elif t < n_pair:
                qkvs[t] = a_project(h, t)
            if 0 <= t - LAG1 < n_pair:
                pvs[t - LAG1] = a_probs(qkvs.pop(t - LAG1))
            if 0 <= t - LAG2 < n_pair:
                outs[t - LAG2] = _dot(*pvs.pop(t - LAG2))
            g = t - LAG3
            if t >= n_pair:
                g = n_pair - LAG3 + (t - n_pair)
            if 0 <= g < n_pair - TAIL:
                y = a_out(outs.pop(g), g)
                acc = y if acc is None else acc + y
        left = sorted(outs)
        o = jnp.concatenate([outs[g] for g in left], axis=1)
        cols = []
        for c in range(nt):
            w = wo_s[left[0]:n_pair, :, c * LANES:(c + 1) * LANES].reshape(-1, LANES)
            cols.append(acc[:, c * LANES:(c + 1) * LANES] + _dot(o, pltpu.bitcast(w, BF16)))
        return a_finish(s, h, jnp.concatenate(cols, axis=1))

    def a_steps(i, mem):
        for u in range(UNROLL):
            mem = a_step(1 + i * UNROLL + u, mem)
        return mem

    assert (n_seg - 1) % UNROLL == 0
    jax.lax.fori_loop(0, (n_seg - 1) // UNROLL, a_steps, a_finish(0, h0, acc0))
    pltpu.make_async_copy(out_vm, out_hbm, out_sem.at[0]).wait()


@functools.partial(jax.jit, static_argnames=("A_seg_len",))
def pallas_gated_mix__memory_aug_recurrent_mem_tr__sliding_local_dilated__prompt_kernel(
    A_x: jax.Array,
    A_mem0: jax.Array,
    A_Wq: jax.Array,
    A_Wk: jax.Array,
    A_Wv: jax.Array,
    A_Wo: jax.Array,
    A_seg_len: int,
    B_x: jax.Array,
    B_wqkv: jax.Array,
    B_wo: jax.Array,
    gate_w: jax.Array,
):
    del B_x
    _, S, D = A_x.shape
    _, H, dh = A_Wq.shape
    M = A_mem0.shape[1]
    PW = 2 * dh
    n_pair = H // 2

    def rows(w):
        return jnp.transpose(w, (1, 2, 0)).reshape(H * dh, D)

    hbm = pl.BlockSpec(memory_space=pl.ANY)
    vmem = pl.BlockSpec(memory_space=pltpu.VMEM)
    out = pl.pallas_call(
        functools.partial(_kernel, seg=int(A_seg_len), dh=dh),
        out_shape=jax.ShapeDtypeStruct((S, D), A_x.dtype),
        in_specs=[hbm, vmem, hbm, hbm, hbm, hbm, hbm, hbm, vmem],
        out_specs=hbm,
        scratch_shapes=[
            pltpu.VMEM((S, D), BF16),
            pltpu.VMEM((3, D, D), BF16),
            pltpu.VMEM((D, D), BF16),
            pltpu.VMEM((3, pl.cdiv(D // 2, LANES), D + 32, LANES), U32),
            pltpu.VMEM((D // LANES, D + 32, LANES), F32),
            pltpu.VMEM((3, D // 2, D), U32),
            pltpu.VMEM((D // 2, D), U32),
            pltpu.VMEM((n_pair, 3, PW // 2, D), U32),
            pltpu.VMEM((n_pair, D // 2, 3 * PW), U32),
            pltpu.VMEM((n_pair, PW // 2, D), U32),
            [pltpu.VMEM((RH, D), F32)] * 2,
            [pltpu.VMEM((D // LANES, HALO + RH, LANES), F32)] * 2,
            [pltpu.VMEM((D // LANES, HALO + RH, LANES), F32)] * 2,
            [pltpu.VMEM((RH, D), BF16)] * 2,
            pltpu.VMEM((S, D), F32),
            pltpu.VMEM((S, D), BF16),
            pltpu.SemaphoreType.DMA((4,)),
            pltpu.SemaphoreType.DMA((S // RB,)),
            pltpu.SemaphoreType.DMA((n_pair, 4)),
            pltpu.SemaphoreType.DMA((1,)),
        ],
        compiler_params=pltpu.CompilerParams(vmem_limit_bytes=110 * 2**20),
    )(A_x.reshape(S, D), A_mem0.reshape(M, D), rows(A_Wq), rows(A_Wk), rows(A_Wv),
      A_Wo.reshape(H * dh, D), B_wqkv, B_wo, gate_w)
    return out.reshape(A_x.shape)
```

```python
import functools

import jax
import jax.numpy as jnp
import jax.experimental.pallas as pl
import jax.experimental.pallas.tpu as pltpu

F32 = jnp.float32
BF16 = jnp.bfloat16
U32 = jnp.uint32
NEG = -1000000000.0

B_HEADS = 32
B_WIN = 8
B_DIL = 2
HALO = 16
RB = 256
RH = RB // 2
RS = 16
LANES = 128
LAG1, LAG2, LAG3 = 1, 4, 8
TAIL = 4
UNROLL = 3


def _iota(shape, dim):
    return jax.lax.broadcasted_iota(jnp.int32, shape, dim)


def _aligned(i, n):
    return i if isinstance(i, int) else pl.multiple_of(i, n)


def _when(cond):
    if isinstance(cond, bool):
        return lambda f: f() if cond else None
    return pl.when(cond)


def _dot(a, b):
    return jnp.dot(a, b, preferred_element_type=F32)


def _dot_nt(a, b):
    return jax.lax.dot_general(a, b, (((1,), (1,)), ((), ())), preferred_element_type=F32)


def _kernel(x_hbm, mem0_ref, wq_hbm, wk_hbm, wv_hbm, wo_hbm, bqkv_hbm, bwo_hbm, gw_ref,
            out_hbm,
            x_vm, bqkv_vm, bwo_vm, perm_s, bwo_t, bqkv_p, bwo_p, stage, wqkv_s, wo_s,
            q_b, k_b, v_b, o_b, b_out, out_vm, in_sem, x_sem, w_sem, out_sem,
            *, seg, dh):
    S, D = x_vm.shape
    M = mem0_ref.shape[0]
    L = M + seg
    n_seg = S // seg
    PW = 2 * dh
    n_pair = wo_hbm.shape[0] // PW
    n_blk = S // RB
    ppb = n_pair // n_blk
    nt = D // LANES
    bdh = D // B_HEADS

    cp_bqkv = [pltpu.make_async_copy(bqkv_hbm.at[:, j * D:(j + 1) * D], bqkv_vm.at[j], in_sem.at[j])
               for j in range(3)]
    cp_bwo = pltpu.make_async_copy(bwo_hbm, bwo_vm, in_sem.at[3])

    def x_copy(i):
        rows = pl.ds(_aligned(i * RB, RB), RB)
        return pltpu.make_async_copy(x_hbm.at[rows, :], x_vm.at[rows, :], x_sem.at[i])

    for c in (cp_bqkv[1], x_copy(0), cp_bqkv[0], cp_bqkv[2], cp_bwo):
        c.start()

    def w_copies(g):
        rows = pl.ds(_aligned(g * (PW // 2), PW // 2), PW // 2)
        dsts = [stage.at[g, 0], stage.at[g, 1], stage.at[g, 2], wo_s.at[g]]
        return [pltpu.make_async_copy(src.bitcast(U32).at[rows, :], dsts[j], w_sem.at[g, j])
                for j, src in enumerate((wq_hbm, wk_hbm, wv_hbm, wo_hbm))]

    def start_batch(i):
        @_when(i + 1 < n_blk)
        def _():
            x_copy(i + 1).start()

        for t in range(ppb):
            for c in w_copies(i * ppb + t):
                c.start()

    def permuted_rows(ref):
        return jnp.concatenate(
            [ref[pl.ds(d, B_HEADS, stride=bdh), :] for d in range(bdh)], axis=0)

    def permute_qkv(j):
        words = pltpu.bitcast(bqkv_vm[j], U32)
        for u, r in enumerate(range(0, D // 2, LANES)):
            n = min(LANES, D // 2 - r)
            blk = words[r:r + n, :]
            if n < LANES:
                blk = jnp.concatenate([blk] * (LANES // n), axis=0)
            perm_s[j, u, 0:D, :] = blk.T
            bqkv_p[j, r:r + n, :] = permuted_rows(perm_s.at[j, u]).T[0:n, :]

    def permute_wo():
        for t in range(nt):
            bwo_t[t, 0:D, :] = bwo_vm[:, t * LANES:(t + 1) * LANES].astype(F32)
            bwo_p[:, t * LANES:(t + 1) * LANES] = pltpu.bitcast(
                permuted_rows(bwo_t.at[t]).astype(BF16), U32)

    a_scale = dh ** -0.5
    half = dh - LANES

    def out_copy(s):
        rows = pl.ds(_aligned(s * seg, seg), seg)
        return pltpu.make_async_copy(out_vm.at[rows, :], out_hbm.at[rows, :], out_sem.at[0])

    def block_diag(a):
        lo = _iota((L, LANES), 1) < half
        z = jnp.zeros((L, LANES), F32)
        mid = a[:, LANES:2 * LANES]
        top = jnp.concatenate([a[:, 0:LANES], jnp.where(lo, mid, 0.0), z], axis=1)
        bot = jnp.concatenate([z, jnp.where(lo, 0.0, mid), a[:, 2 * LANES:3 * LANES]], axis=1)
        return jnp.concatenate([top, bot], axis=0).astype(BF16)

    def a_rows(s, mem):
        row0 = _aligned(s * seg, seg)
        return jnp.concatenate([mem, x_vm[pl.ds(row0, seg), :].astype(F32)], axis=0)

    def a_project(h, g):
        return _dot(h, pltpu.bitcast(wqkv_s[g], BF16))

    def a_probs(qkv):
        row = _iota((L, 2 * L), 0)
        col = _iota((L, 2 * L), 1)
        first = col < L
        visible = (row < M) | (row >= jnp.where(first, col, col - L))
        sc = _dot_nt(qkv[:, 0:PW], block_diag(qkv[:, PW:2 * PW])) * a_scale
        sc = jnp.where(visible, sc, NEG)
        m0 = jnp.max(jnp.where(first, sc, -jnp.inf), axis=1, keepdims=True)
        m1 = jnp.max(jnp.where(first, -jnp.inf, sc), axis=1, keepdims=True)
        e = jnp.exp(sc - jnp.where(first, m0, m1))
        s0 = jnp.sum(jnp.where(first, e, 0.0), axis=1, keepdims=True)
        s1 = jnp.sum(jnp.where(first, 0.0, e), axis=1, keepdims=True)
        return e / jnp.where(first, s0, s1), block_diag(qkv[:, 2 * PW:3 * PW])

    def a_out(o, g):
        return _dot(o, pltpu.bitcast(wo_s[g], BF16))

    def a_finish(s, h, acc):
        rows = pl.ds(_aligned(s * seg, seg), seg)
        gw = gw_ref[...].astype(F32).reshape(1, D)
        z = jnp.sum(h[M:, :] * gw, axis=1, keepdims=True)
        g = 1.0 / (1.0 + jnp.exp(-z))
        out_vm[rows, :] = (g * acc[M:, :] + (1.0 - g) * b_out[rows, :]).astype(BF16)
        out_copy(s).start()
        return acc[0:M, :]

    b_scale = bdh ** -0.5

    def relayout(g):
        for j in range(3):
            wt = pltpu.bitcast(stage[g, j], BF16).T
            wqkv_s[g, :, j * PW:(j + 1) * PW] = pltpu.bitcast(wt, U32)

    def b_project(c, u, parts=(1, 0, 2)):
        xb = x_vm[pl.ds(_aligned(c * RH, RH), RH), :]
        for j in parts:
            y = _dot(xb, pltpu.bitcast(bqkv_p[j], BF16))
            if j == 0:
                q_b[u][...] = y * b_scale
            else:
                for t in range(nt):
                    (k_b, v_b)[j - 1][u][t, HALO:HALO + RH, :] = y[:, t * LANES:(t + 1) * LANES]

    def b_halo(u, first=False):
        for buf in (k_b, v_b):
            for t in range(nt):
                if first:
                    tail = jnp.broadcast_to(buf[u][t, HALO:HALO + 1, :], (HALO, LANES))
                else:
                    tail = buf[1 - u][t, RH:RH + HALO, :]
                buf[u][t, 0:HALO, :] = tail

    def b_attend(u, first=False):
        for r in range(0, RH, RS):
            base = HALO + r
            qs = [q_b[u][r:r + RS, t * LANES:(t + 1) * LANES] for t in range(nt)]
            logits = []
            for w in range(B_WIN):
                lo = base - w * B_DIL
                acc = qs[0] * k_b[u][0, lo:lo + RS, :]
                for t in range(1, nt):
                    acc = acc + qs[t] * k_b[u][t, lo:lo + RS, :]
                acc = acc + pltpu.roll(acc, 2 * B_HEADS, 1)
                acc = acc + pltpu.roll(acc, B_HEADS, 1)
                if first and r < w * B_DIL:
                    acc = jnp.where(r + _iota((RS, LANES), 0) >= w * B_DIL, acc, NEG)
                logits.append(acc)
            mx = functools.reduce(jnp.maximum, logits)
            es = [jnp.exp(l - mx) for l in logits]
            inv = 1.0 / functools.reduce(jnp.add, es)
            ps = [e * inv for e in es]
            for t in range(nt):
                acc = ps[0] * v_b[u][t, base:base + RS, :]
                for w in range(1, B_WIN):
                    lo = base - w * B_DIL
                    acc = acc + ps[w] * v_b[u][t, lo:lo + RS, :]
                o_b[u][r:r + RS, t * LANES:(t + 1) * LANES] = acc.astype(BF16)

    def b_finish(c, u):
        rows = pl.ds(_aligned(c * RH, RH), RH)
        b_out[rows, :] = _dot(o_b[u][...], pltpu.bitcast(bwo_p[...], BF16))

    def fetch(i):
        x_copy(i).wait()

        @_when(i + 1 < n_blk)
        def _():
            start_batch(i + 1)

    def arrived(i):
        gs = [i * ppb + t for t in range(ppb)]
        for g in gs:
            for c in w_copies(g):
                c.wait()
        return gs

    def b_block(i, acc):
        gs = arrived(i - 1)
        fetch(i)
        h = a_rows(0, mem0_ref[...].astype(F32))
        b_halo(1)
        b_attend(1)
        b_project(2 * i, 0)
        for g in gs:
            relayout(g)
        b_finish(2 * i - 2, 0)
        b_halo(0)
        b_attend(0)
        qkvs = [a_project(h, g) for g in gs]
        pvs = [a_probs(qkv) for qkv in qkvs]
        b_project(2 * i + 1, 1)
        outs = [_dot(*pv) for pv in pvs]
        b_finish(2 * i - 1, 1)
        for g, o in zip(gs, outs):
            acc = acc + a_out(o, g)
        return acc

    cp_bqkv[1].wait()
    permute_qkv(1)
    start_batch(0)
    x_copy(0).wait()
    cp_bqkv[0].wait()
    permute_qkv(0)
    b_project(0, 0, (1,))
    b_project(1, 1, (1,))
    cp_bqkv[2].wait()
    cp_bwo.wait()
    permute_qkv(2)
    b_project(0, 0, (0,))
    b_project(1, 1, (0,))
    start_batch(1)
    permute_wo()
    b_project(0, 0, (2,))
    b_halo(0, first=True)
    b_attend(0, first=True)
    b_project(1, 1, (2,))
    acc0 = jax.lax.fori_loop(1, n_blk, b_block, jnp.zeros((L, D), F32))
    gs = arrived(n_blk - 1)
    h0 = a_rows(0, mem0_ref[...].astype(F32))
    for g in gs:
        relayout(g)
    b_halo(1)
    b_attend(1)
    b_finish(2 * n_blk - 2, 0)
    qkvs = [a_project(h0, g) for g in gs]
    pvs = [a_probs(qkv) for qkv in qkvs]
    b_finish(2 * n_blk - 1, 1)
    outs = [_dot(*pv) for pv in pvs]
    for g, o in zip(gs, outs):
        acc0 = acc0 + a_out(o, g)

    def a_step(s, mem):
        h = a_rows(s, mem)
        qkvs, pvs, outs, acc = {}, {}, {}, None
        for t in range(n_pair + LAG2):
            if t == 0:
                qkvs[t] = functools.reduce(jnp.add, [
                    _dot(h[:, c * LANES:(c + 1) * LANES],
                         pltpu.bitcast(wqkv_s[t, c * LANES // 2:(c + 1) * LANES // 2, :], BF16))
                    for c in range(nt)])
            elif t < n_pair:
                qkvs[t] = a_project(h, t)
            if 0 <= t - LAG1 < n_pair:
                pvs[t - LAG1] = a_probs(qkvs.pop(t - LAG1))
            if 0 <= t - LAG2 < n_pair:
                outs[t - LAG2] = _dot(*pvs.pop(t - LAG2))
            g = t - LAG3
            if t >= n_pair:
                g = n_pair - LAG3 + (t - n_pair)
            if 0 <= g < n_pair - TAIL:
                y = a_out(outs.pop(g), g)
                acc = y if acc is None else acc + y
        left = sorted(outs)
        o = jnp.concatenate([outs[g] for g in left], axis=1)
        cols = []
        for c in range(nt):
            w = wo_s[left[0]:n_pair, :, c * LANES:(c + 1) * LANES].reshape(-1, LANES)
            cols.append(acc[:, c * LANES:(c + 1) * LANES] + _dot(o, pltpu.bitcast(w, BF16)))
        return a_finish(s, h, jnp.concatenate(cols, axis=1))

    def a_steps(i, mem):
        for u in range(UNROLL):
            mem = a_step(1 + i * UNROLL + u, mem)
        return mem

    assert (n_seg - 1) % UNROLL == 0
    jax.lax.fori_loop(0, (n_seg - 1) // UNROLL, a_steps, a_finish(0, h0, acc0))
    pltpu.make_async_copy(out_vm, out_hbm, out_sem.at[0]).wait()


@functools.partial(jax.jit, static_argnames=("A_seg_len",))
def pallas_gated_mix__memory_aug_recurrent_mem_tr__sliding_local_dilated__prompt_kernel(
    A_x: jax.Array,
    A_mem0: jax.Array,
    A_Wq: jax.Array,
    A_Wk: jax.Array,
    A_Wv: jax.Array,
    A_Wo: jax.Array,
    A_seg_len: int,
    B_x: jax.Array,
    B_wqkv: jax.Array,
    B_wo: jax.Array,
    gate_w: jax.Array,
):
    del B_x
    _, S, D = A_x.shape
    _, H, dh = A_Wq.shape
    M = A_mem0.shape[1]
    PW = 2 * dh
    n_pair = H // 2

    def rows(w):
        return jnp.transpose(w, (1, 2, 0)).reshape(H * dh, D)

    hbm = pl.BlockSpec(memory_space=pl.ANY)
    vmem = pl.BlockSpec(memory_space=pltpu.VMEM)
    out = pl.pallas_call(
        functools.partial(_kernel, seg=int(A_seg_len), dh=dh),
        out_shape=jax.ShapeDtypeStruct((S, D), A_x.dtype),
        in_specs=[hbm, vmem, hbm, hbm, hbm, hbm, hbm, hbm, vmem],
        out_specs=hbm,
        scratch_shapes=[
            pltpu.VMEM((S, D), BF16),
            pltpu.VMEM((3, D, D), BF16),
            pltpu.VMEM((D, D), BF16),
            pltpu.VMEM((3, pl.cdiv(D // 2, LANES), D + 32, LANES), U32),
            pltpu.VMEM((D // LANES, D + 32, LANES), F32),
            pltpu.VMEM((3, D // 2, D), U32),
            pltpu.VMEM((D // 2, D), U32),
            pltpu.VMEM((n_pair, 3, PW // 2, D), U32),
            pltpu.VMEM((n_pair, D // 2, 3 * PW), U32),
            pltpu.VMEM((n_pair, PW // 2, D), U32),
            [pltpu.VMEM((RH, D), F32)] * 2,
            [pltpu.VMEM((D // LANES, HALO + RH, LANES), F32)] * 2,
            [pltpu.VMEM((D // LANES, HALO + RH, LANES), F32)] * 2,
            [pltpu.VMEM((RH, D), BF16)] * 2,
            pltpu.VMEM((S, D), F32),
            pltpu.VMEM((S, D), BF16),
            pltpu.SemaphoreType.DMA((4,)),
            pltpu.SemaphoreType.DMA((S // RB,)),
            pltpu.SemaphoreType.DMA((n_pair, 4)),
            pltpu.SemaphoreType.DMA((1,)),
        ],
        compiler_params=pltpu.CompilerParams(vmem_limit_bytes=110 * 2**20),
    )(A_x.reshape(S, D), A_mem0.reshape(M, D), rows(A_Wq), rows(A_Wk), rows(A_Wv),
      A_Wo.reshape(H * dh, D), B_wqkv, B_wo, gate_w)
    return out.reshape(A_x.shape)
```

```python
import functools

import jax
import jax.numpy as jnp
import jax.experimental.pallas as pl
import jax.experimental.pallas.tpu as pltpu

F32 = jnp.float32
BF16 = jnp.bfloat16
U32 = jnp.uint32
NEG = -1000000000.0

B_HEADS = 32
B_WIN = 8
B_DIL = 2
HALO = 16
RB = 256
RH = RB // 2
RS = 16
LANES = 128
LAG1, LAG2, LAG3 = 1, 4, 8
TAIL = 4
UNROLL = 3


def _iota(shape, dim):
    return jax.lax.broadcasted_iota(jnp.int32, shape, dim)


def _aligned(i, n):
    return i if isinstance(i, int) else pl.multiple_of(i, n)


def _when(cond):
    if isinstance(cond, bool):
        return lambda f: f() if cond else None
    return pl.when(cond)


def _dot(a, b):
    return jnp.dot(a, b, preferred_element_type=F32)


def _dot_nt(a, b):
    return jax.lax.dot_general(a, b, (((1,), (1,)), ((), ())), preferred_element_type=F32)


def _kernel(x_hbm, mem0_ref, wq_hbm, wk_hbm, wv_hbm, wo_hbm, bqkv_hbm, bwo_hbm, gw_ref,
            out_hbm,
            x_vm, bqkv_vm, bwo_vm, perm_s, bwo_t, bqkv_p, bwo_p, stage, wqkv_s, wo_s,
            q_b, k_b, v_b, o_b, b_out, out_vm, in_sem, x_sem, w_sem, out_sem,
            *, seg, dh):
    S, D = x_vm.shape
    M = mem0_ref.shape[0]
    L = M + seg
    n_seg = S // seg
    PW = 2 * dh
    n_pair = wo_hbm.shape[0]
    n_blk = S // RB
    ppb = n_pair // n_blk
    nt = D // LANES
    bdh = D // B_HEADS

    cp_bqkv = [pltpu.make_async_copy(bqkv_hbm.at[:, j * D:(j + 1) * D], bqkv_vm.at[j], in_sem.at[j])
               for j in range(3)]
    cp_bwo = pltpu.make_async_copy(bwo_hbm, bwo_vm, in_sem.at[3])

    def x_copy(i):
        rows = pl.ds(_aligned(i * RB, RB), RB)
        return pltpu.make_async_copy(x_hbm.at[rows, :], x_vm.at[rows, :], x_sem.at[i])

    for c in (cp_bqkv[1], x_copy(0), cp_bqkv[0], cp_bqkv[2], cp_bwo):
        c.start()

    def w_copies(i):
        gs = pl.ds(i * ppb, ppb)
        dsts = [stage.at[0], stage.at[1], stage.at[2], wo_s]
        return [pltpu.make_async_copy(src.bitcast(U32).at[gs], dsts[j].at[gs], w_sem.at[i, j])
                for j, src in enumerate((wq_hbm, wk_hbm, wv_hbm, wo_hbm))]

    def start_batch(i):
        @_when(i + 1 < n_blk)
        def _():
            x_copy(i + 1).start()

        for c in w_copies(i):
            c.start()

    def permuted_rows(ref):
        return jnp.concatenate(
            [ref[pl.ds(d, B_HEADS, stride=bdh), :] for d in range(bdh)], axis=0)

    def permute_qkv(j):
        words = pltpu.bitcast(bqkv_vm[j], U32)
        for u, r in enumerate(range(0, D // 2, LANES)):
            n = min(LANES, D // 2 - r)
            blk = words[r:r + n, :]
            if n < LANES:
                blk = jnp.concatenate([blk] * (LANES // n), axis=0)
            perm_s[j, u, 0:D, :] = blk.T
            bqkv_p[j, r:r + n, :] = permuted_rows(perm_s.at[j, u]).T[0:n, :]

    def permute_wo():
        for t in range(nt):
            bwo_t[t, 0:D, :] = bwo_vm[:, t * LANES:(t + 1) * LANES].astype(F32)
            bwo_p[:, t * LANES:(t + 1) * LANES] = pltpu.bitcast(
                permuted_rows(bwo_t.at[t]).astype(BF16), U32)

    a_scale = dh ** -0.5
    half = dh - LANES

    def out_copy(s):
        rows = pl.ds(_aligned(s * seg, seg), seg)
        return pltpu.make_async_copy(out_vm.at[rows, :], out_hbm.at[rows, :], out_sem.at[0])

    def block_diag(a):
        lo = _iota((L, LANES), 1) < half
        z = jnp.zeros((L, LANES), F32)
        mid = a[:, LANES:2 * LANES]
        top = jnp.concatenate([a[:, 0:LANES], jnp.where(lo, mid, 0.0), z], axis=1)
        bot = jnp.concatenate([z, jnp.where(lo, 0.0, mid), a[:, 2 * LANES:3 * LANES]], axis=1)
        return jnp.concatenate([top, bot], axis=0).astype(BF16)

    def a_rows(s, mem):
        row0 = _aligned(s * seg, seg)
        return jnp.concatenate([mem, x_vm[pl.ds(row0, seg), :].astype(F32)], axis=0)

    def a_project(h, g):
        return _dot(h, pltpu.bitcast(wqkv_s[g], BF16))

    def a_probs(qkv):
        row = _iota((L, 2 * L), 0)
        col = _iota((L, 2 * L), 1)
        first = col < L
        visible = (row < M) | (row >= jnp.where(first, col, col - L))
        sc = _dot_nt(qkv[:, 0:PW], block_diag(qkv[:, PW:2 * PW])) * a_scale
        sc = jnp.where(visible, sc, NEG)
        m0 = jnp.max(jnp.where(first, sc, -jnp.inf), axis=1, keepdims=True)
        m1 = jnp.max(jnp.where(first, -jnp.inf, sc), axis=1, keepdims=True)
        e = jnp.exp(sc - jnp.where(first, m0, m1))
        s0 = jnp.sum(jnp.where(first, e, 0.0), axis=1, keepdims=True)
        s1 = jnp.sum(jnp.where(first, 0.0, e), axis=1, keepdims=True)
        return e / jnp.where(first, s0, s1), block_diag(qkv[:, 2 * PW:3 * PW])

    def a_out(o, g):
        return _dot(o, pltpu.bitcast(wo_s[g], BF16))

    def a_finish(s, h, acc):
        rows = pl.ds(_aligned(s * seg, seg), seg)
        gw = gw_ref[...].astype(F32).reshape(1, D)
        z = jnp.sum(h[M:, :] * gw, axis=1, keepdims=True)
        g = 1.0 / (1.0 + jnp.exp(-z))
        out_vm[rows, :] = (g * acc[M:, :] + (1.0 - g) * b_out[rows, :]).astype(BF16)
        out_copy(s).start()
        return acc[0:M, :]

    b_scale = bdh ** -0.5

    def relayout(g):
        for j in range(3):
            wt = pltpu.bitcast(stage[j, g], BF16).T
            wqkv_s[g, :, j * PW:(j + 1) * PW] = pltpu.bitcast(wt, U32)

    def b_project(c, u, parts=(1, 0, 2)):
        xb = x_vm[pl.ds(_aligned(c * RH, RH), RH), :]
        for j in parts:
            y = _dot(xb, pltpu.bitcast(bqkv_p[j], BF16))
            if j == 0:
                q_b[u][...] = y * b_scale
            else:
                for t in range(nt):
                    (k_b, v_b)[j - 1][u][t, HALO:HALO + RH, :] = y[:, t * LANES:(t + 1) * LANES]

    def b_halo(u, first=False):
        for buf in (k_b, v_b):
            for t in range(nt):
                if first:
                    tail = jnp.broadcast_to(buf[u][t, HALO:HALO + 1, :], (HALO, LANES))
                else:
                    tail = buf[1 - u][t, RH:RH + HALO, :]
                buf[u][t, 0:HALO, :] = tail

    def b_attend(u, first=False):
        for r in range(0, RH, RS):
            base = HALO + r
            qs = [q_b[u][r:r + RS, t * LANES:(t + 1) * LANES] for t in range(nt)]
            logits = []
            for w in range(B_WIN):
                lo = base - w * B_DIL
                acc = qs[0] * k_b[u][0, lo:lo + RS, :]
                for t in range(1, nt):
                    acc = acc + qs[t] * k_b[u][t, lo:lo + RS, :]
                acc = acc + pltpu.roll(acc, 2 * B_HEADS, 1)
                acc = acc + pltpu.roll(acc, B_HEADS, 1)
                if first and r < w * B_DIL:
                    acc = jnp.where(r + _iota((RS, LANES), 0) >= w * B_DIL, acc, NEG)
                logits.append(acc)
            mx = functools.reduce(jnp.maximum, logits)
            es = [jnp.exp(l - mx) for l in logits]
            inv = 1.0 / functools.reduce(jnp.add, es)
            ps = [e * inv for e in es]
            for t in range(nt):
                acc = ps[0] * v_b[u][t, base:base + RS, :]
                for w in range(1, B_WIN):
                    lo = base - w * B_DIL
                    acc = acc + ps[w] * v_b[u][t, lo:lo + RS, :]
                o_b[u][r:r + RS, t * LANES:(t + 1) * LANES] = acc.astype(BF16)

    def b_finish(c, u):
        rows = pl.ds(_aligned(c * RH, RH), RH)
        b_out[rows, :] = _dot(o_b[u][...], pltpu.bitcast(bwo_p[...], BF16))

    def fetch(i):
        x_copy(i).wait()

        @_when(i + 1 < n_blk)
        def _():
            start_batch(i + 1)

    def arrived(i):
        for c in w_copies(i):
            c.wait()
        return [i * ppb + t for t in range(ppb)]

    def b_block(i, acc):
        gs = arrived(i - 1)
        fetch(i)
        h = a_rows(0, mem0_ref[...].astype(F32))
        b_halo(1)
        b_attend(1)
        b_project(2 * i, 0)
        for g in gs:
            relayout(g)
        b_finish(2 * i - 2, 0)
        b_halo(0)
        b_attend(0)
        qkvs = [a_project(h, g) for g in gs]
        pvs = [a_probs(qkv) for qkv in qkvs]
        b_project(2 * i + 1, 1)
        outs = [_dot(*pv) for pv in pvs]
        b_finish(2 * i - 1, 1)
        for g, o in zip(gs, outs):
            acc = acc + a_out(o, g)
        return acc

    cp_bqkv[1].wait()
    permute_qkv(1)
    start_batch(0)
    x_copy(0).wait()
    cp_bqkv[0].wait()
    permute_qkv(0)
    b_project(0, 0, (1,))
    b_project(1, 1, (1,))
    cp_bqkv[2].wait()
    cp_bwo.wait()
    permute_qkv(2)
    b_project(0, 0, (0,))
    b_project(1, 1, (0,))
    permute_wo()
    b_project(0, 0, (2,))
    b_halo(0, first=True)
    b_attend(0, first=True)
    b_project(1, 1, (2,))
    start_batch(1)
    acc0 = jax.lax.fori_loop(1, n_blk, b_block, jnp.zeros((L, D), F32))
    gs = arrived(n_blk - 1)
    h0 = a_rows(0, mem0_ref[...].astype(F32))
    for g in gs:
        relayout(g)
    b_halo(1)
    b_attend(1)
    b_finish(2 * n_blk - 2, 0)
    qkvs = [a_project(h0, g) for g in gs]
    pvs = [a_probs(qkv) for qkv in qkvs]
    b_finish(2 * n_blk - 1, 1)
    outs = [_dot(*pv) for pv in pvs]
    for g, o in zip(gs, outs):
        acc0 = acc0 + a_out(o, g)

    def a_step(s, mem):
        h = a_rows(s, mem)
        qkvs, pvs, outs, acc = {}, {}, {}, None
        for t in range(n_pair + LAG2):
            if t == 0:
                qkvs[t] = functools.reduce(jnp.add, [
                    _dot(h[:, c * LANES:(c + 1) * LANES],
                         pltpu.bitcast(wqkv_s[t, c * LANES // 2:(c + 1) * LANES // 2, :], BF16))
                    for c in range(nt)])
            elif t < n_pair:
                qkvs[t] = a_project(h, t)
            if 0 <= t - LAG1 < n_pair:
                pvs[t - LAG1] = a_probs(qkvs.pop(t - LAG1))
            if 0 <= t - LAG2 < n_pair:
                outs[t - LAG2] = _dot(*pvs.pop(t - LAG2))
            g = t - LAG3
            if t >= n_pair:
                g = n_pair - LAG3 + (t - n_pair)
            if 0 <= g < n_pair - TAIL:
                y = a_out(outs.pop(g), g)
                acc = y if acc is None else acc + y
        left = sorted(outs)
        o = jnp.concatenate([outs[g] for g in left], axis=1)
        cols = []
        for c in range(nt):
            w = wo_s[left[0]:n_pair, :, c * LANES:(c + 1) * LANES].reshape(-1, LANES)
            cols.append(acc[:, c * LANES:(c + 1) * LANES] + _dot(o, pltpu.bitcast(w, BF16)))
        return a_finish(s, h, jnp.concatenate(cols, axis=1))

    def a_steps(i, mem):
        for u in range(UNROLL):
            mem = a_step(1 + i * UNROLL + u, mem)
        return mem

    assert (n_seg - 1) % UNROLL == 0
    jax.lax.fori_loop(0, (n_seg - 1) // UNROLL, a_steps, a_finish(0, h0, acc0))
    pltpu.make_async_copy(out_vm, out_hbm, out_sem.at[0]).wait()


@functools.partial(jax.jit, static_argnames=("A_seg_len",))
def pallas_gated_mix__memory_aug_recurrent_mem_tr__sliding_local_dilated__prompt_kernel(
    A_x: jax.Array,
    A_mem0: jax.Array,
    A_Wq: jax.Array,
    A_Wk: jax.Array,
    A_Wv: jax.Array,
    A_Wo: jax.Array,
    A_seg_len: int,
    B_x: jax.Array,
    B_wqkv: jax.Array,
    B_wo: jax.Array,
    gate_w: jax.Array,
):
    del B_x
    _, S, D = A_x.shape
    _, H, dh = A_Wq.shape
    M = A_mem0.shape[1]
    PW = 2 * dh
    n_pair = H // 2

    def rows(w):
        return jnp.transpose(w, (1, 2, 0)).reshape(n_pair, PW, D)

    hbm = pl.BlockSpec(memory_space=pl.ANY)
    vmem = pl.BlockSpec(memory_space=pltpu.VMEM)
    out = pl.pallas_call(
        functools.partial(_kernel, seg=int(A_seg_len), dh=dh),
        out_shape=jax.ShapeDtypeStruct((S, D), A_x.dtype),
        in_specs=[hbm, vmem, hbm, hbm, hbm, hbm, hbm, hbm, vmem],
        out_specs=hbm,
        scratch_shapes=[
            pltpu.VMEM((S, D), BF16),
            pltpu.VMEM((3, D, D), BF16),
            pltpu.VMEM((D, D), BF16),
            pltpu.VMEM((3, pl.cdiv(D // 2, LANES), D + 32, LANES), U32),
            pltpu.VMEM((D // LANES, D + 32, LANES), F32),
            pltpu.VMEM((3, D // 2, D), U32),
            pltpu.VMEM((D // 2, D), U32),
            pltpu.VMEM((3, n_pair, PW // 2, D), U32),
            pltpu.VMEM((n_pair, D // 2, 3 * PW), U32),
            pltpu.VMEM((n_pair, PW // 2, D), U32),
            [pltpu.VMEM((RH, D), F32)] * 2,
            [pltpu.VMEM((D // LANES, HALO + RH, LANES), F32)] * 2,
            [pltpu.VMEM((D // LANES, HALO + RH, LANES), F32)] * 2,
            [pltpu.VMEM((RH, D), BF16)] * 2,
            pltpu.VMEM((S, D), F32),
            pltpu.VMEM((S, D), BF16),
            pltpu.SemaphoreType.DMA((4,)),
            pltpu.SemaphoreType.DMA((S // RB,)),
            pltpu.SemaphoreType.DMA((S // RB, 4)),
            pltpu.SemaphoreType.DMA((1,)),
        ],
        compiler_params=pltpu.CompilerParams(vmem_limit_bytes=110 * 2**20),
    )(A_x.reshape(S, D), A_mem0.reshape(M, D), rows(A_Wq), rows(A_Wk), rows(A_Wv),
      A_Wo.reshape(n_pair, PW, D), B_wqkv, B_wo, gate_w)
    return out.reshape(A_x.shape)
```

```python
import functools

import jax
import jax.numpy as jnp
import jax.experimental.pallas as pl
import jax.experimental.pallas.tpu as pltpu

F32 = jnp.float32
BF16 = jnp.bfloat16
U32 = jnp.uint32
NEG = -1000000000.0

B_HEADS = 32
B_WIN = 8
B_DIL = 2
HALO = 16
RB = 256
RH = RB // 2
RS = 16
LANES = 128
LAG1, LAG2, LAG3 = 1, 4, 8
TAIL = 4
UNROLL = 3


def _iota(shape, dim):
    return jax.lax.broadcasted_iota(jnp.int32, shape, dim)


def _aligned(i, n):
    return i if isinstance(i, int) else pl.multiple_of(i, n)


def _when(cond):
    if isinstance(cond, bool):
        return lambda f: f() if cond else None
    return pl.when(cond)


def _dot(a, b):
    return jnp.dot(a, b, preferred_element_type=F32)


def _dot_nt(a, b):
    return jax.lax.dot_general(a, b, (((1,), (1,)), ((), ())), preferred_element_type=F32)


def _kernel(x_hbm, mem0_ref, wq_hbm, wk_hbm, wv_hbm, wo_hbm, bqkv_hbm, bwo_hbm, gw_ref,
            out_hbm,
            x_vm, bqkv_vm, bwo_vm, perm_s, bwo_t, bqkv_p, bwo_p, stage, wqkv_s, wo_s,
            q_b, k_b, v_b, o_b, b_out, out_vm, in_sem, x_sem, w_sem, out_sem,
            *, seg, dh):
    S, D = x_vm.shape
    M = mem0_ref.shape[0]
    L = M + seg
    n_seg = S // seg
    PW = 2 * dh
    n_pair = wo_hbm.shape[0]
    n_blk = S // RB
    ppb = n_pair // n_blk
    nt = D // LANES
    bdh = D // B_HEADS

    cp_bqkv = [pltpu.make_async_copy(bqkv_hbm.at[:, j * D:(j + 1) * D], bqkv_vm.at[j], in_sem.at[j])
               for j in range(3)]
    cp_bwo = pltpu.make_async_copy(bwo_hbm, bwo_vm, in_sem.at[3])

    def x_copy(i):
        rows = pl.ds(_aligned(i * RB, RB), RB)
        return pltpu.make_async_copy(x_hbm.at[rows, :], x_vm.at[rows, :], x_sem.at[i])

    for c in (cp_bqkv[1], x_copy(0), cp_bqkv[0], cp_bqkv[2], cp_bwo):
        c.start()

    def w_copies(i):
        gs = pl.ds(i * ppb, ppb)
        return [pltpu.make_async_copy(src.at[gs], stage.at[j, gs], w_sem.at[i, j])
                for j, src in enumerate((wq_hbm, wk_hbm, wv_hbm, wo_hbm))]

    def start_batch(i):
        @_when(i + 1 < n_blk)
        def _():
            x_copy(i + 1).start()

        for c in w_copies(i):
            c.start()

    def permuted_rows(ref):
        return jnp.concatenate(
            [ref[pl.ds(d, B_HEADS, stride=bdh), :] for d in range(bdh)], axis=0)

    def permute_qkv(j):
        words = pltpu.bitcast(bqkv_vm[j], U32)
        for u, r in enumerate(range(0, D // 2, LANES)):
            n = min(LANES, D // 2 - r)
            blk = words[r:r + n, :]
            if n < LANES:
                blk = jnp.concatenate([blk] * (LANES // n), axis=0)
            perm_s[j, u, 0:D, :] = blk.T
            bqkv_p[j, r:r + n, :] = permuted_rows(perm_s.at[j, u]).T[0:n, :]

    def permute_wo():
        for t in range(nt):
            bwo_t[t, 0:D, :] = bwo_vm[:, t * LANES:(t + 1) * LANES].astype(F32)
            bwo_p[:, t * LANES:(t + 1) * LANES] = pltpu.bitcast(
                permuted_rows(bwo_t.at[t]).astype(BF16), U32)

    a_scale = dh ** -0.5
    half = dh - LANES

    def out_copy(s):
        rows = pl.ds(_aligned(s * seg, seg), seg)
        return pltpu.make_async_copy(out_vm.at[rows, :], out_hbm.at[rows, :], out_sem.at[0])

    def block_diag(a):
        lo = _iota((L, LANES), 1) < half
        z = jnp.zeros((L, LANES), F32)
        mid = a[:, LANES:2 * LANES]
        top = jnp.concatenate([a[:, 0:LANES], jnp.where(lo, mid, 0.0), z], axis=1)
        bot = jnp.concatenate([z, jnp.where(lo, 0.0, mid), a[:, 2 * LANES:3 * LANES]], axis=1)
        return jnp.concatenate([top, bot], axis=0).astype(BF16)

    def a_rows(s, mem):
        row0 = _aligned(s * seg, seg)
        return jnp.concatenate([mem, x_vm[pl.ds(row0, seg), :].astype(F32)], axis=0)

    def a_project(h, g):
        return _dot(h, pltpu.bitcast(wqkv_s[g], BF16))

    def a_probs(qkv):
        row = _iota((L, 2 * L), 0)
        col = _iota((L, 2 * L), 1)
        first = col < L
        visible = (row < M) | (row >= jnp.where(first, col, col - L))
        sc = _dot_nt(qkv[:, 0:PW], block_diag(qkv[:, PW:2 * PW])) * a_scale
        sc = jnp.where(visible, sc, NEG)
        m0 = jnp.max(jnp.where(first, sc, -jnp.inf), axis=1, keepdims=True)
        m1 = jnp.max(jnp.where(first, -jnp.inf, sc), axis=1, keepdims=True)
        e = jnp.exp(sc - jnp.where(first, m0, m1))
        s0 = jnp.sum(jnp.where(first, e, 0.0), axis=1, keepdims=True)
        s1 = jnp.sum(jnp.where(first, 0.0, e), axis=1, keepdims=True)
        return e / jnp.where(first, s0, s1), block_diag(qkv[:, 2 * PW:3 * PW])

    def a_out(o, g):
        return _dot(o, pltpu.bitcast(wo_s[g], BF16))

    def a_finish(s, h, acc):
        rows = pl.ds(_aligned(s * seg, seg), seg)
        gw = gw_ref[...].astype(F32).reshape(1, D)
        z = jnp.sum(h[M:, :] * gw, axis=1, keepdims=True)
        g = 1.0 / (1.0 + jnp.exp(-z))
        out_vm[rows, :] = (g * acc[M:, :] + (1.0 - g) * b_out[rows, :]).astype(BF16)
        out_copy(s).start()
        return acc[0:M, :]

    b_scale = bdh ** -0.5

    def relayout(g):
        for j in range(3):
            wt = stage[j, g].T
            wqkv_s[g, :, j * PW:(j + 1) * PW] = pltpu.bitcast(wt, U32)
        wo_s[g] = pltpu.bitcast(stage[3, g], U32)

    def b_project(c, u, parts=(1, 0, 2)):
        xb = x_vm[pl.ds(_aligned(c * RH, RH), RH), :]
        for j in parts:
            y = _dot(xb, pltpu.bitcast(bqkv_p[j], BF16))
            if j == 0:
                q_b[u][...] = y * b_scale
            else:
                for t in range(nt):
                    (k_b, v_b)[j - 1][u][t, HALO:HALO + RH, :] = y[:, t * LANES:(t + 1) * LANES]

    def b_halo(u, first=False):
        for buf in (k_b, v_b):
            for t in range(nt):
                if first:
                    tail = jnp.broadcast_to(buf[u][t, HALO:HALO + 1, :], (HALO, LANES))
                else:
                    tail = buf[1 - u][t, RH:RH + HALO, :]
                buf[u][t, 0:HALO, :] = tail

    def b_attend(u, first=False):
        for r in range(0, RH, RS):
            base = HALO + r
            qs = [q_b[u][r:r + RS, t * LANES:(t + 1) * LANES] for t in range(nt)]
            logits = []
            for w in range(B_WIN):
                lo = base - w * B_DIL
                acc = qs[0] * k_b[u][0, lo:lo + RS, :]
                for t in range(1, nt):
                    acc = acc + qs[t] * k_b[u][t, lo:lo + RS, :]
                acc = acc + pltpu.roll(acc, 2 * B_HEADS, 1)
                acc = acc + pltpu.roll(acc, B_HEADS, 1)
                if first and r < w * B_DIL:
                    acc = jnp.where(r + _iota((RS, LANES), 0) >= w * B_DIL, acc, NEG)
                logits.append(acc)
            mx = functools.reduce(jnp.maximum, logits)
            es = [jnp.exp(l - mx) for l in logits]
            inv = 1.0 / functools.reduce(jnp.add, es)
            ps = [e * inv for e in es]
            for t in range(nt):
                acc = ps[0] * v_b[u][t, base:base + RS, :]
                for w in range(1, B_WIN):
                    lo = base - w * B_DIL
                    acc = acc + ps[w] * v_b[u][t, lo:lo + RS, :]
                o_b[u][r:r + RS, t * LANES:(t + 1) * LANES] = acc.astype(BF16)

    def b_finish(c, u):
        rows = pl.ds(_aligned(c * RH, RH), RH)
        b_out[rows, :] = _dot(o_b[u][...], pltpu.bitcast(bwo_p[...], BF16))

    def fetch(i):
        x_copy(i).wait()

        @_when(i + 1 < n_blk)
        def _():
            start_batch(i + 1)

    def arrived(i):
        for c in w_copies(i):
            c.wait()
        return [i * ppb + t for t in range(ppb)]

    def b_block(i, acc):
        gs = arrived(i - 1)
        fetch(i)
        h = a_rows(0, mem0_ref[...].astype(F32))
        b_halo(1)
        b_attend(1)
        b_project(2 * i, 0)
        for g in gs:
            relayout(g)
        b_finish(2 * i - 2, 0)
        b_halo(0)
        b_attend(0)
        qkvs = [a_project(h, g) for g in gs]
        pvs = [a_probs(qkv) for qkv in qkvs]
        b_project(2 * i + 1, 1)
        outs = [_dot(*pv) for pv in pvs]
        b_finish(2 * i - 1, 1)
        for g, o in zip(gs, outs):
            acc = acc + a_out(o, g)
        return acc

    cp_bqkv[1].wait()
    permute_qkv(1)
    start_batch(0)
    x_copy(0).wait()
    cp_bqkv[0].wait()
    permute_qkv(0)
    b_project(0, 0, (1,))
    b_project(1, 1, (1,))
    cp_bqkv[2].wait()
    cp_bwo.wait()
    permute_qkv(2)
    b_project(0, 0, (0,))
    b_project(1, 1, (0,))
    permute_wo()
    b_project(0, 0, (2,))
    b_halo(0, first=True)
    b_attend(0, first=True)
    b_project(1, 1, (2,))
    start_batch(1)
    acc0 = jax.lax.fori_loop(1, n_blk, b_block, jnp.zeros((L, D), F32))
    gs = arrived(n_blk - 1)
    h0 = a_rows(0, mem0_ref[...].astype(F32))
    for g in gs:
        relayout(g)
    b_halo(1)
    b_attend(1)
    b_finish(2 * n_blk - 2, 0)
    qkvs = [a_project(h0, g) for g in gs]
    pvs = [a_probs(qkv) for qkv in qkvs]
    b_finish(2 * n_blk - 1, 1)
    outs = [_dot(*pv) for pv in pvs]
    for g, o in zip(gs, outs):
        acc0 = acc0 + a_out(o, g)

    def a_step(s, mem):
        h = a_rows(s, mem)
        qkvs, pvs, outs, acc = {}, {}, {}, None
        for t in range(n_pair + LAG2):
            if t == 0:
                qkvs[t] = functools.reduce(jnp.add, [
                    _dot(h[:, c * LANES:(c + 1) * LANES],
                         pltpu.bitcast(wqkv_s[t, c * LANES // 2:(c + 1) * LANES // 2, :], BF16))
                    for c in range(nt)])
            elif t < n_pair:
                qkvs[t] = a_project(h, t)
            if 0 <= t - LAG1 < n_pair:
                pvs[t - LAG1] = a_probs(qkvs.pop(t - LAG1))
            if 0 <= t - LAG2 < n_pair:
                outs[t - LAG2] = _dot(*pvs.pop(t - LAG2))
            g = t - LAG3
            if t >= n_pair:
                g = n_pair - LAG3 + (t - n_pair)
            if 0 <= g < n_pair - TAIL:
                y = a_out(outs.pop(g), g)
                acc = y if acc is None else acc + y
        left = sorted(outs)
        o = jnp.concatenate([outs[g] for g in left], axis=1)
        cols = []
        for c in range(nt):
            w = wo_s[left[0]:n_pair, :, c * LANES:(c + 1) * LANES].reshape(-1, LANES)
            cols.append(acc[:, c * LANES:(c + 1) * LANES] + _dot(o, pltpu.bitcast(w, BF16)))
        return a_finish(s, h, jnp.concatenate(cols, axis=1))

    def a_steps(i, mem):
        for u in range(UNROLL):
            mem = a_step(1 + i * UNROLL + u, mem)
        return mem

    assert (n_seg - 1) % UNROLL == 0
    jax.lax.fori_loop(0, (n_seg - 1) // UNROLL, a_steps, a_finish(0, h0, acc0))
    pltpu.make_async_copy(out_vm, out_hbm, out_sem.at[0]).wait()


@functools.partial(jax.jit, static_argnames=("A_seg_len",))
def pallas_gated_mix__memory_aug_recurrent_mem_tr__sliding_local_dilated__prompt_kernel(
    A_x: jax.Array,
    A_mem0: jax.Array,
    A_Wq: jax.Array,
    A_Wk: jax.Array,
    A_Wv: jax.Array,
    A_Wo: jax.Array,
    A_seg_len: int,
    B_x: jax.Array,
    B_wqkv: jax.Array,
    B_wo: jax.Array,
    gate_w: jax.Array,
):
    del B_x
    _, S, D = A_x.shape
    _, H, dh = A_Wq.shape
    M = A_mem0.shape[1]
    PW = 2 * dh
    n_pair = H // 2

    def rows(w):
        return jnp.transpose(w, (1, 2, 0)).reshape(n_pair, PW, D)

    hbm = pl.BlockSpec(memory_space=pl.ANY)
    vmem = pl.BlockSpec(memory_space=pltpu.VMEM)
    out = pl.pallas_call(
        functools.partial(_kernel, seg=int(A_seg_len), dh=dh),
        out_shape=jax.ShapeDtypeStruct((S, D), A_x.dtype),
        in_specs=[hbm, vmem, hbm, hbm, hbm, hbm, hbm, hbm, vmem],
        out_specs=hbm,
        scratch_shapes=[
            pltpu.VMEM((S, D), BF16),
            pltpu.VMEM((3, D, D), BF16),
            pltpu.VMEM((D, D), BF16),
            pltpu.VMEM((3, pl.cdiv(D // 2, LANES), D + 32, LANES), U32),
            pltpu.VMEM((D // LANES, D + 32, LANES), F32),
            pltpu.VMEM((3, D // 2, D), U32),
            pltpu.VMEM((D // 2, D), U32),
            pltpu.VMEM((4, n_pair, PW, D), BF16),
            pltpu.VMEM((n_pair, D // 2, 3 * PW), U32),
            pltpu.VMEM((n_pair, PW // 2, D), U32),
            [pltpu.VMEM((RH, D), F32)] * 2,
            [pltpu.VMEM((D // LANES, HALO + RH, LANES), F32)] * 2,
            [pltpu.VMEM((D // LANES, HALO + RH, LANES), F32)] * 2,
            [pltpu.VMEM((RH, D), BF16)] * 2,
            pltpu.VMEM((S, D), F32),
            pltpu.VMEM((S, D), BF16),
            pltpu.SemaphoreType.DMA((4,)),
            pltpu.SemaphoreType.DMA((S // RB,)),
            pltpu.SemaphoreType.DMA((S // RB, 4)),
            pltpu.SemaphoreType.DMA((1,)),
        ],
        compiler_params=pltpu.CompilerParams(vmem_limit_bytes=110 * 2**20),
    )(A_x.reshape(S, D), A_mem0.reshape(M, D), rows(A_Wq), rows(A_Wk), rows(A_Wv),
      A_Wo.reshape(n_pair, PW, D), B_wqkv, B_wo, gate_w)
    return out.reshape(A_x.shape)
```
